```python
import os as _os
_os.environ.setdefault("JAX_PLATFORMS", "cpu")
import jax
import jax.numpy as jnp

def _softmax(x, axis=-1):
    return jax.nn.softmax(x, axis=axis)
def _gelu(x):
    return jax.nn.gelu(x, approximate=True)
def _silu(x):
    return jax.nn.silu(x)
def _sigmoid(x):
    return jax.nn.sigmoid(x)
def _layernorm(x, axis=-1, eps=1e-5):
    m = jnp.mean(x, axis=axis, keepdims=True)
    v = jnp.var(x, axis=axis, keepdims=True)
    return (x - m) / jnp.sqrt(v + eps)
def _scatter_add(tgt, idx, src, axis=0):
    return tgt.at[idx].add(src)
def _segment_sum(src, seg, n):
    return jax.ops.segment_sum(src, seg, n)
class _Rng:
    def __init__(self, key):
        self._k = key
    def _next(self):
        self._k, sub = jax.random.split(self._k)
        return sub
    def normal(self, shape):
        return jax.random.normal(self._next(), shape, dtype=jnp.bfloat16)
    def randint(self, lo, hi, shape):
        return jax.random.randint(self._next(), shape, lo, hi, dtype=jnp.int32)
    def uniform(self, shape, lo=0.0, hi=1.0):
        return jax.random.uniform(self._next(), shape, jnp.bfloat16, lo, hi)
    def permutation(self, n):
        return jax.random.permutation(self._next(), n)


kernel_name = 'gated_mix__ssm_conv_h3__mixer_s_mlp__prompt'

def setup_inputs():
    _rng = _Rng(jax.random.key(int.from_bytes(__import__("os").urandom(4), "little")))
    _w = (lambda a: (lambda t: t.astype(jnp.bfloat16) if jnp.issubdtype(t.dtype, jnp.floating) else t)(jnp.asarray(a)))
    def _A_setup():
        B, S, D = 1, 2048, 576
        ks = 4
        return {
            "q": _w((lambda *s: _rng.normal(s) * 0.05)(B, S, D)),
            "k": _w((lambda *s: _rng.normal(s) * 0.4)(B, S, D)),
            "v": _w((lambda *s: _rng.normal(s) * 0.4)(B, S, D)),
            "shift_k": _w((lambda *s: _rng.normal(s) * 0.4)(D, ks) * 0.5),
            "ssm_k": _w((lambda *s: _rng.normal(s) * 0.4)(D, S) * (1.0 / S ** 0.5)),
            "ssm_D": _w((lambda *s: _rng.normal(s) * 0.4)(D)),
        }
    _A_in = _A_setup()

    def _B_setup():
        B, S, D, F = 1, 2048, 576, 4608
        return {
            "x":  _w((lambda *s: _rng.normal(s) * 0.05)(B, S, D)),
            "w1": _w((lambda *s: _rng.normal(s) * 0.2)(D, D) * (D ** -0.5)),
            "w2": _w((lambda *s: _rng.normal(s) * 0.2)(D, D) * (D ** -0.5)),
            "w3": _w((lambda *s: _rng.normal(s) * 0.2)(D, F) * (D ** -0.5)),
            "w4": _w((lambda *s: _rng.normal(s) * 0.2)(F, D) * (F ** -0.5)),
        }
    _B_in = _B_setup()

    return {
        "A_q": _A_in["q"],
        "A_k": _A_in["k"],
        "A_v": _A_in["v"],
        "A_shift_k": _A_in["shift_k"],
        "A_ssm_k": _A_in["ssm_k"],
        "A_ssm_D": _A_in["ssm_D"],
        "B_x": _B_in["x"],
        "B_w1": _B_in["w1"],
        "B_w2": _B_in["w2"],
        "B_w3": _B_in["w3"],
        "B_w4": _B_in["w4"],
        "gate_w": _w((lambda *s: _rng.normal(s) * 0.05)(576) * 16.0),
    }

def reference(A_q, A_k, A_v, A_shift_k, A_ssm_k, A_ssm_D, B_x, B_w1, B_w2, B_w3, B_w4, gate_w):
    def _A_ref(q, k, v, shift_k, ssm_k, ssm_D):
        B, S, D = q.shape
        ks = shift_k.shape[-1]
        k_pad = jnp.pad(k, ((0, 0), (ks - 1, 0), (0, 0)))
        k_shift = jnp.zeros_like(k)
        for t in range(ks):
            k_shift = k_shift + k_pad[:, t:t + S, :] * shift_k[:, ks - 1 - t][None, None, :]
        kv = k_shift * v
        L = 2 * S
        kv_pad = jnp.pad(kv, ((0, 0), (0, S), (0, 0)))
        kf_pad = jnp.pad(ssm_k, ((0, 0), (0, S)))
        kv_f = (lambda x, axes=(-2,-1): jnp.fft.rfft2(x.astype(jnp.float32), axes=axes))(kv_pad[:, None, :, :], axes=(1, 2))
        kf_f = (lambda x, axes=(-2,-1): jnp.fft.rfft2(x.astype(jnp.float32), axes=axes))(kf_pad[:, None, :], axes=(1, 2))
        kf_f = (lambda x, *d: x.transpose(*d))(kf_f, 1, 2, 0)
        y_f = kv_f * kf_f[None, :, :, :]
        y = (lambda x, s, axes=(-2,-1): jnp.fft.irfft2(x, s=s, axes=axes).astype(jnp.bfloat16))(y_f, (1, L), axes=(1, 2))[:, 0, :S, :]
        y = y + kv * ssm_D[None, None, :]
        return q * y

    def _B_ref(x, w1, w2, w3, w4):
        B, S, D = x.shape
        h = _gelu(_layernorm(x, axis=-1) @ w1)
        c = D // 4
        g0 = jnp.pad(h[:, :, 0*c:1*c], ((0, 0), (1, 0), (0, 0)))[:, :S, :]
        g1 = jnp.pad(h[:, :, 1*c:2*c], ((0, 0), (0, 1), (0, 0)))[:, 1:, :]
        g2 = jnp.pad(h[:, :, 2*c:3*c], ((0, 0), (2, 0), (0, 0)))[:, :S, :]
        g3 = jnp.pad(h[:, :, 3*c:   ], ((0, 0), (0, 2), (0, 0)))[:, 2:, :]
        hs = jnp.concatenate([g0, g1, g2, g3], axis=-1) @ w2
        x1 = x + hs
        h2 = _gelu(_layernorm(x1, axis=-1) @ w3) @ w4
        return x1 + h2

    x = A_q
    g = _sigmoid((x * gate_w).sum(-1, keepdims=True))
    a = _A_ref(x, A_k, A_v, A_shift_k, A_ssm_k, A_ssm_D)
    b = _B_ref(x, B_w1, B_w2, B_w3, B_w4)
    return g * a + (1 - g) * b
```

```python
import functools
import math

import jax
import jax.numpy as jnp
import numpy as np
from jax import lax
from jax.experimental import pallas as pl
from jax.experimental.pallas import tpu as pltpu

def cfg(k, d):
    return d
S, D, F = 2048, 576, 4608
KS = 4
EPS = 1e-5
LANES = 128

NB, NP = 4, 49
NH = (NP + 1) // 2
FC = 512
NF = F // FC
TB = 1024
NT = S // TB
TS = TB // NB
KM = 512
KS3 = KM // NB
FS = FC // NB
DS = D // NB
STEPS = NF * NT

W3_ROWS = NH * KS3 + NB * NB // 2 * (D - KM)
W4_ROWS = NH * DS

NC = S // LANES
CG = D // STEPS

GELU_C0 = math.sqrt(2.0 / math.pi)
GELU_C1 = GELU_C0 * 0.044715

f32, bf16, u32 = jnp.float32, jnp.bfloat16, jnp.uint32
_NN = (((1,), (0,)), ((), ()))
_NT = (((1,), (1,)), ((), ()))

_AC = [{(0, 0): 1, (1, 1): 1}, {(1, 0): 1, (1, 1): 1}, {(0, 0): 1}, {(1, 1): 1},
       {(0, 0): 1, (0, 1): 1}, {(1, 0): 1, (0, 0): -1}, {(0, 1): 1, (1, 1): -1}]
_BC = [{(0, 0): 1, (1, 1): 1}, {(0, 0): 1}, {(0, 1): 1, (1, 1): -1}, {(1, 0): 1, (0, 0): -1},
       {(1, 1): 1}, {(0, 0): 1, (0, 1): 1}, {(1, 0): 1, (1, 1): 1}]
_CC = [{(0, 0): 1, (1, 1): 1}, {(1, 0): 1, (1, 1): -1}, {(0, 1): 1, (1, 1): 1},
       {(0, 0): 1, (1, 0): 1}, {(0, 0): -1, (0, 1): 1}, {(1, 1): 1}, {(0, 0): 1}]


_TAIL1 = {6: (0, (0, 1)), 5: (1, (0, 1)), 1: (1, (0,)), 4: (0, (1,))}
_TAIL = {7 * i + j: (2 * bi + bj, tuple(2 * u + v for u in ci for v in cj))
         for i, (bi, ci) in _TAIL1.items() for j, (bj, cj) in _TAIL1.items()}
_TAIL_SLOT = {prod: n for n, prod in enumerate(sorted(_TAIL))}


def _dft_matrix():
    n = np.arange(LANES)[:, None]
    f = np.arange(LANES)[None, :]
    theta = np.pi * (((2 * f + 1) * n) % (4 * LANES)) / (2 * LANES)
    return np.concatenate([np.cos(theta), -np.sin(theta)], axis=1).astype(jnp.bfloat16)


def _mm(a, b, dims=_NN):
    return lax.dot_general(a, b, dims, preferred_element_type=f32)


def _gelu2(x):
    u = x * (x * x * GELU_C1 + GELU_C0)
    return x * jnp.tanh(u) + x


def _combine(blocks, coef):
    n = len(blocks) // 2
    out = []
    for r in range(n):
        row = []
        for c in range(n):
            acc = None
            for (r0, c0), sign in coef.items():
                v = blocks[r0 * n + r][c0 * n + c]
                acc = v if acc is None else (acc + v if sign > 0 else acc - v)
            row.append(acc)
        out.append(row)
    return out


def _gather(get, levels, base=0, init=None):
    if levels == 0:
        return [[get(base)]]
    r, n = 7 ** (levels - 1), 2 ** (levels - 1)
    out = [[None] * (2 * n) for _ in range(2 * n)] if init is None else [list(x) for x in init]
    for i in (0, 1, 2, 3, 5, 6, 4):
        m = _gather(get, levels - 1, base + i * r)
        for (r0, c0), sign in _CC[i].items():
            for a in range(n):
                for c in range(n):
                    o = out[r0 * n + a][c0 * n + c]
                    if o is None:
                        o = m[a][c]
                    else:
                        o = o + m[a][c] if sign > 0 else o - m[a][c]
                    out[r0 * n + a][c0 * n + c] = o
    return out


def _interleave(*streams):
    streams = [s for s in streams if s]
    total = [float(sum(w for w, _ in s)) for s in streams]
    pos, done = [0] * len(streams), [0.0] * len(streams)
    while True:
        live = [k for k in range(len(streams)) if pos[k] < len(streams[k])]
        if not live:
            return
        k = min(live, key=lambda j: (done[j] + 0.5 * streams[j][pos[j]][0]) / total[j])
        w, fn = streams[k][pos[k]]
        pos[k] += 1
        done[k] += w
        fn()


def _merge(*streams):
    out = []
    _interleave(*[[(sum(w for w, _ in grp), functools.partial(out.extend, grp)) for grp in s] for s in streams])
    return out


def _singles(stream):
    return [[t] for t in stream]


def _kernel(q_hbm, k_hbm, v_hbm, shift_hbm, ssm_hbm, dd_hbm, w1_hbm, w2_hbm, w3_hbm, w4_hbm,
            gw_hbm, dft_hbm, o_hbm,
            q_v, w1_v, w2_v, w3_v, w4_v, shift_v, dd_v, gw_v, dft_v, o_v,
            k_a, k_b, v_a, v_b, s_a, s_b, p_a, p_b,
            w1t_u, w2t_u, dft_u, pcol, gate, x1, xn_u, h1_u, xt, xc_u, xl_u,
            w3c_u, w4c_u,
            acc, z_a, z_b, h_a, h_b, kv_a, kv_b, xf_a, xf_b, kf_a, kf_b, zf_a, zf_b,
            abuf, sems, idle):
    w1t, w2t, dft = w1t_u.bitcast(bf16), w2t_u.bitcast(bf16), dft_u.bitcast(bf16)
    xn, h1, xl = xn_u.bitcast(bf16), h1_u.bitcast(bf16), xl_u.bitcast(bf16)
    xc = [xc_u.at[pl.ds(t * NH * TS // 2, NH * TS // 2), :].bitcast(bf16) for t in range(NT)]
    z = (z_a, z_b)
    h = (h_a.bitcast(bf16), h_b.bitcast(bf16))
    kv = (kv_a.bitcast(bf16), kv_b.bitcast(bf16))
    xf, kf, mb = (xf_a, xf_b), (kf_a, kf_b), (zf_a, zf_b)
    kg, vg, sg, pg = (k_a, k_b), (v_a, v_b), (s_a, s_b), (p_a, p_b)
    task = functools.partial

    T1 = 512
    n1 = S // T1
    sem_ids = iter(range(sems.shape[0]))

    def copy(src, dst):
        return pltpu.make_async_copy(src, dst, sems.at[next(sem_ids)])

    cp_q = [copy(q_hbm.at[:, pl.ds(T1 * i, T1)], q_v.at[:, pl.ds(T1 * i, T1)]) for i in range(n1)]
    cp_w1, cp_w2 = copy(w1_hbm, w1_v), copy(w2_hbm, w2_v)
    cp_small = [copy(shift_hbm, shift_v), copy(dd_hbm, dd_v), copy(gw_hbm, gw_v), copy(dft_hbm, dft_v)]
    sem_w3, sem_w4 = (sems.at[next(sem_ids)] for _ in range(2))
    sem_conv = [[sems.at[next(sem_ids)] for _ in range(4)] for _ in range(2)]

    def fetch_w3(f):
        return pltpu.make_async_copy(w3_hbm.at[:, rows_at(f * FC, 0, FC, FC)], w3_v, sem_w3)

    def fetch_w4(f):
        return pltpu.make_async_copy(w4_hbm.at[:, rows_at(f * FC, 0, FC, FC)], w4_v, sem_w4)

    def fetch_group(g, p):
        rows = rows_at(g * CG, 0, CG)
        srcs = (k_hbm.at[rows, :], v_hbm.at[rows, :], ssm_hbm.at[rows, :],
                pcol.at[rows, pl.ds(0, (KS + 1) * LANES)])
        return [pltpu.make_async_copy(src, dst[p], sem)
                for src, dst, sem in zip(srcs, (kg, vg, sg, pg), sem_conv[p])]

    def start(cps):
        for cp in cps:
            cp.start()

    def wait(cps):
        for cp in cps:
            cp.wait()

    TO = TB // 2
    cp_o = [copy(o_v.at[:, pl.ds(TO * i, TO)], o_hbm.at[:, pl.ds(TO * i, TO)]) for i in range(S // TO)]

    def rows_at(base, offset, size, align=16):
        if isinstance(base, int):
            return pl.ds(base + offset, size)
        return pl.ds(pl.multiple_of(base + offset, align), size)

    def paired(i, height, offset, size):
        return pl.ds(i // 2 * height + offset, size), pl.ds(i % 2 * LANES, LANES)

    def tail_rows(n, offset, size):
        return paired(n, D - KM, NH * KS3 + offset, size)

    def chunks(ref_u32, first_row, rows, count):
        window = ref_u32.at[rows_at(first_row, 0, count * (rows // 2), 8), :]
        return [window.at[pl.ds(i * (rows // 2), rows // 2), :].bitcast(bf16) for i in range(count)]

    def product(i, offset, size):
        return paired(i, TS, offset, size)

    head, tail_blocks = [], []

    def transpose_tasks(src, dst):
        ts = []
        for c0 in range(0, D, LANES):
            c1 = min(D, c0 + LANES)

            def t(c0=c0, c1=c1):
                dst[c0:c1, :] = src[:, c0:c1].T
            ts.append((1, t))
        return ts

    def param_tasks():
        def column(j):
            row = (shift_v[j:j + 1, :].astype(f32) if j < KS
                   else (dd_v, gw_v)[j - KS][...].astype(f32).reshape(1, D))
            pcol[:, pl.ds(j * LANES, LANES)] = jnp.broadcast_to(row, (LANES, D)).T

        def mat():
            dft[...] = dft_v[...]

        def pad():
            zero = jnp.zeros((D // 2, LANES), u32)
            h1_u[:, 0:LANES] = zero
            h1_u[:, LANES + S:] = zero
        return [(1, task(column, j)) for j in range(KS + 2)] + [(1, mat), (1, pad)]

    def rstd_of(c):
        cs = pl.ds(c * LANES, LANES)
        mean = jnp.sum(x1[:, cs], axis=0, keepdims=True) * (1.0 / D)
        d = x1[:, cs] - mean
        var = jnp.sum(d * d, axis=0, keepdims=True) * (1.0 / D)
        return mean, lax.rsqrt(var + EPS)

    def ln0_tasks(b):
        ts = []
        for c in range(b * T1 // LANES, (b + 1) * T1 // LANES):
            cs = pl.ds(c * LANES, LANES)

            def t(c=c, cs=cs):
                x1[:, cs] = q_v[:, cs].astype(f32)
                mean, rstd = rstd_of(c)
                xn[:, cs] = ((x1[:, cs] - mean) * rstd).astype(bf16)
            ts.append((1, t))
        return ts

    def gate_tasks(b):
        ts = []
        for c in range(b * T1 // LANES, (b + 1) * T1 // LANES):
            cs = pl.ds(c * LANES, LANES)

            def t(cs=cs):
                s = jnp.sum(q_v[:, cs].astype(f32) * pcol[:, pl.ds((KS + 1) * LANES, LANES)], axis=0, keepdims=True)
                gate[:, cs] = jnp.broadcast_to(jax.nn.sigmoid(s), (8, LANES))
            ts.append((1, t))
        return ts

    def h1_tasks(b):
        ts = []
        for c in range(b * T1 // LANES, (b + 1) * T1 // LANES):
            def t(c=c):
                y = _mm(w1t[...], xn[:, pl.ds(c * LANES, LANES)])
                h1[:, pl.ds((c + 1) * LANES, LANES)] = (0.5 * _gelu2(y)).astype(bf16)
            ts.append((1, t))
        return ts

    def hs_tasks(b):
        ts = []
        rows = D // 8
        for c in range(b * T1 // LANES, (b + 1) * T1 // LANES):
            def t(c=c):
                parts = [
                    pltpu.bitcast(h1_u[pl.ds(g * rows, rows), pl.ds((c + 1) * LANES - dlt, LANES)], bf16)
                    for g, dlt in enumerate((1, -1, 2, -2))]
                cs = pl.ds(c * LANES, LANES)
                x1[:, cs] += _mm(w2t[...], jnp.concatenate(parts, axis=0))
            ts.append((1, t))
        return ts

    def ln1_tasks(t):
        ts = []
        for c in range(t * TB // LANES, (t + 1) * TB // LANES):
            def norm(c=c):
                mean, rstd = rstd_of(c)
                cs = pl.ds(c * LANES, LANES)
                xt[cs, pl.ds(0, D)] = ((x1[:, cs] - mean) * rstd).T
            ts.append((1, norm))
        return ts

    def xc_tasks(t):
        ts = []
        for r in range(TS // 16):
            def combos(r=r):
                for b in range(NB):
                    rs = pl.ds(t * TB + b * TS + r * 16, 16)
                    xl[rs, pl.ds(0, D - KM)] = xt[rs, pl.ds(KM, D - KM)].astype(bf16)
                blk = [[xt[pl.ds(t * TB + b * TS + r * 16, 16), pl.ds(k * KS3, KS3)]
                        for k in range(NB)] for b in range(NB)]
                for i in range(7):
                    mid = _combine(blk, _AC[i])
                    for j in range(7):
                        xc[t][product(7 * i + j, r * 16, 16)] = _combine(mid, _AC[j])[0][0].astype(bf16)
            ts.append((1, combos))
        return ts

    def w3_combo_tasks(w3s):
        ts = []
        for r in range(KS3 // 16):
            def combos(r=r):
                if r < (D - KM) // 16:
                    tail = [w3_v[pl.ds(KM + r * 16, 16), pl.ds(a * FS, FS)].astype(f32) for a in range(NB)]
                    for prod, n in _TAIL_SLOT.items():
                        w3s[tail_rows(n, r * 16, 16)] = functools.reduce(
                            lambda x, y: x + y, [tail[a] for a in _TAIL[prod][1]]).astype(bf16)
                blk = [[w3_v[pl.ds(k * KS3 + r * 16, 16), pl.ds(a * FS, FS)].astype(f32)
                        for a in range(NB)] for k in range(NB)]
                for i in range(7):
                    mid = _combine(blk, _BC[i])
                    for j in range(7):
                        w3s[paired(7 * i + j, KS3, r * 16, 16)] = _combine(mid, _BC[j])[0][0].astype(bf16)
            ts.append((200, combos))
        return ts

    def w4_combo_tasks(w4s):
        ts = []
        for r in range(DS // 16):
            def combos(r=r):
                blk = [[w4_v[pl.ds(a * DS + r * 16, 16), pl.ds(b * FS, FS)].astype(f32)
                        for b in range(NB)] for a in range(NB)]
                for i in range(7):
                    mid = _combine(blk, _AC[i])
                    for j in range(7):
                        w4s[paired(7 * i + j, DS, r * 16, 16)] = _combine(mid, _AC[j])[0][0].astype(bf16)
            ts.append((200, combos))
        return ts

    def zero_tasks(t):
        def zero(i):
            acc[t, i] = jnp.zeros((DS, TS), f32)
        return [(1, task(zero, i)) for i in range(NP)]

    def z_tasks(w3c, t):
        ts = []
        for i in range(NP):
            def prod(i=i):
                y = _mm(xc[t][product(i, 0, TS)], w3c[paired(i, KS3, 0, KS3)])
                if i in _TAIL:
                    y = y + _mm(xl[pl.ds(t * TB + _TAIL[i][0] * TS, TS), pl.ds(0, D - KM)],
                                w3c[tail_rows(_TAIL_SLOT[i], 0, D - KM)])
                z[t][product(i, 0, TS)] = y
            ts.append((TS * (2 if i in _TAIL else 1), prod))
        return ts

    def act_tasks(t):
        ts = []
        for r in range(TS // 16):
            st = {}

            def half(k, r=r, st=st):
                r0 = r * 16 + k * 8
                pre = _gather(lambda i: z[t][product(i, r0, 8)], 2)
                st[k] = [[_gelu2(pre[b][a]) for b in range(NB)] for a in range(NB)]
            grp = [(192, task(half, 0)), (192, task(half, 1))]
            for i in range(7):
                def combos(i=i, r=r, st=st):
                    lo, hi = _combine(st[0], _BC[i]), _combine(st[1], _BC[i])
                    for j in range(7):
                        v = jnp.concatenate(
                            [_combine(lo, _BC[j])[0][0], _combine(hi, _BC[j])[0][0]], axis=0)
                        h[t][product(7 * i + j, r * 16, 16)] = v.astype(bf16)
                grp.append((32, combos))
            ts.append(grp)
        return ts

    def w_tasks(w4c, t):
        ts = []
        for i in range(NP):
            def prod(i=i):
                acc[t, i] += _mm(w4c[paired(i, DS, 0, DS)], h[t][product(i, 0, TS)], _NT)
            ts.append((DS * TS // LANES, prod))
        return ts

    def group_rows(g):
        return rows_at(g * CG, 0, CG)

    def kv_tasks(p):
        ts = []
        W = 512
        for c in range(S // W):
            def t(c=c):
                taps = [jnp.tile(pg[p][:, pl.ds(j * LANES, LANES)], (1, W // LANES)) for j in range(KS)]
                if c == 0:
                    kk = jnp.concatenate([jnp.zeros((CG, LANES), f32), kg[p][:, 0:W].astype(f32)], axis=1)
                else:
                    kk = kg[p][:, pl.ds(c * W - LANES, W + LANES)].astype(f32)
                ksum = kk[:, LANES:] * taps[0]
                for j in range(1, KS):
                    ksum = ksum + kk[:, LANES - j:LANES - j + W] * taps[j]
                prod = (ksum * vg[p][:, pl.ds(c * W, W)].astype(f32)).astype(bf16)
                for i in range(W // LANES):
                    j = c * W // LANES + i
                    kv[p][pl.ds(j % (NC // 2) * CG, CG), pl.ds(j // (NC // 2) * LANES, LANES)] = (
                        prod[:, i * LANES:(i + 1) * LANES])
            ts.append((150, t))
        return ts

    def fwd_tasks(p):
        ts = []
        half = NC // 2
        for part in range(2):
            dst = pl.ds(part * half * CG, half * CG)

            def data(part=part, dst=dst):
                xf[p][dst, :] = _mm(kv[p][:, pl.ds(part * LANES, LANES)], dft[...])

            def filt(part=part, dst=dst):
                lhs = jnp.concatenate(
                    [sg[p][:, pl.ds(j * LANES, LANES)] for j in range(part * half, (part + 1) * half)], axis=0)
                y = _mm(lhs, dft[...])
                if part == 0:
                    kf[p][0:CG, 0:LANES] = y[0:CG, 0:LANES] + pg[p][:, pl.ds(KS * LANES, LANES)]
                    kf[p][0:CG, LANES:] = y[0:CG, LANES:]
                    kf[p][CG:half * CG, :] = y[CG:]
                else:
                    kf[p][dst, :] = y
            ts += [(2 * half * CG, data), (2 * half * CG, filt)]
        return ts

    def mac_tasks(g, p):
        ts = []
        IB = cfg("ib", 2)
        zero = (g // (2 * STEPS)) * 8 if not isinstance(g, int) else 0
        if not cfg("order", 0):
            zero = 0

        def stage(u, j, e):
            return NC * CG + (u % 2) * 2 * NC * 8 + j * 16 + e // 2 * 8, pl.ds(e % 2 * LANES, LANES)

        def ld(u, j, e):
            row, col = stage(u, j, e)
            return mb[p][rows_at(zero, row, 8, 8), col]

        for u in range(CG // 8):
            def spec(ref, j, u=u):
                rs = pl.ds(j * CG + u * 8, 8)
                return ref[rs, 0:LANES], ref[rs, LANES:]

            def prep(u=u, spec=spec):
                lane = lax.broadcasted_iota(jnp.int32, (8, LANES), 1)
                sgn = jnp.where(lane % 2 == 0, 1.0, -1.0).astype(f32)
                prev = None
                for j in range(NC):
                    cur = c, d = spec(kf[p], j)
                    if prev is not None:
                        c, d = c - sgn * prev[1], d + sgn * prev[0]
                    prev = cur
                    a, b = spec(xf[p], j)
                    for e, val in enumerate((c, d - c, c + d, a + b)):
                        row, col = stage(u, j, e)
                        mb[p][pl.ds(row, 8), col] = val
            ts.append((NC * 7, prep))
            for i0 in range(0, NC, IB):
                def block_out(i0=i0, u=u, spec=spec):
                    sums = {i: None for i in range(i0, i0 + IB)}
                    xs = {}
                    for m in range(i0 + IB):
                        ks = [ld(u, m, e) for e in range(3)]
                        for i in range(max(i0, m), i0 + IB):
                            if i - m not in xs:
                                xs[i - m] = (ld(u, i - m, 3),) + spec(xf[p], i - m)
                            terms = [kk * xx for kk, xx in zip(ks, xs[i - m])]
                            sums[i] = terms if sums[i] is None else [s + t for s, t in zip(sums[i], terms)]
                    for i in range(i0, i0 + IB):
                        a1, a2, a3 = sums[i]
                        mb[p][pl.ds(i * CG + u * 8, 8), 0:LANES] = a1 - a3
                        mb[p][pl.ds(i * CG + u * 8, 8), LANES:] = a1 + a2
                ts.append((6 * sum(i + 1 for i in range(i0, i0 + IB)), block_out))
        return ts

    def inv_tasks(row, p):
        qg, ag = q_v.at[rows_at(row, 0, CG), :], abuf.at[rows_at(row, 0, CG), :]
        ts = []
        half = NC // 2
        for part in range(2):
            def t(part=part):
                y = _mm(mb[p][pl.ds(part * half * CG, half * CG), :].astype(bf16), dft[...], _NT)
                for j in range(half):
                    cs = pl.ds((part * half + j) * LANES, LANES)
                    ag[:, cs] = y[j * CG:(j + 1) * CG] * qg[:, cs].astype(f32)
            ts.append((2 * half * CG, t))
        return ts

    def out_tasks(t, bs):
        ts = []
        for c in range(TS // LANES):
            for r in range(DS // 16):
                def o(r=r, c=c):
                    cs = pl.ds(c * LANES, LANES)
                    blk = _gather(lambda i: acc[t, i, pl.ds(r * 16, 16), cs], 2)
                    for b in bs:
                        tok = pl.ds(t * TB + b * TS + c * LANES, LANES)
                        g8 = gate[:, tok]
                        g = jnp.concatenate([g8, g8], axis=0)
                        for a in range(NB):
                            rs = pl.ds(a * DS + r * 16, 16)
                            mlp = x1[rs, tok] + 0.5 * blk[a][b]
                            o_v[rs, tok] = (g * (abuf[rs, tok] * (1.0 / LANES))
                                            + (1.0 - g) * mlp).astype(bf16)
                ts.append((1, o))
        return ts

    cp_q[0].start()
    cp_w1.start()
    start(cp_small)
    cp_q[1].start()
    w3_first, w4_first = chunks(w3c_u, 0, W3_ROWS, 2), chunks(w4c_u, 0, W4_ROWS, 1)
    w4_last = chunks(w4c_u, (NF - 1) * W4_ROWS // 2, W4_ROWS, 1)[0]

    @head.append
    def _():
        wait([cp_q[0], cp_w1])
        start([cp_w2] + cp_q[2:])

    @head.append
    def _():
        _interleave(transpose_tasks(w1_v, w1t), ln0_tasks(0))

    @head.append
    def _():
        wait(cp_small + [cp_q[1]])
        start([fetch_w3(0), fetch_w4(0)])

    @head.append
    def _():
        _interleave(h1_tasks(0), ln0_tasks(1), param_tasks())

    @head.append
    def _():
        wait([cp_q[2], cp_w2])
        start(fetch_group(0, 0) + fetch_group(1, 1))

    @head.append
    def _():
        _interleave(h1_tasks(1), ln0_tasks(2), transpose_tasks(w2_v, w2t), gate_tasks(0))

    @head.append
    def _():
        wait([cp_q[3], fetch_w3(0)])

    @head.append
    def _():
        _interleave(h1_tasks(2), ln0_tasks(3), gate_tasks(1), w3_combo_tasks(w3_first[0]))

    @head.append
    def _():
        wait([fetch_w4(0)])
        start([fetch_w3(1)])

    @head.append
    def _():
        _interleave(h1_tasks(3), gate_tasks(2), w4_combo_tasks(w4_first[0]))

    @head.append
    def _():
        wait([fetch_w3(1)])
        start([fetch_w4(1)])

    @head.append
    def _():
        _interleave(hs_tasks(0) + hs_tasks(1), gate_tasks(3), w3_combo_tasks(w3_first[1]), zero_tasks(0))

    @head.append
    def _():
        wait(fetch_group(0, 0))

    @head.append
    def _():
        _interleave(hs_tasks(2) + hs_tasks(3), ln1_tasks(0) + xc_tasks(0), kv_tasks(0))
        _interleave(fwd_tasks(0))

    @head.append
    def _():
        start(fetch_group(2, 0))

    @head.append
    def _():
        _interleave(z_tasks(w3_first[0], 0), ln1_tasks(1) + xc_tasks(1), zero_tasks(1))

    @head.append
    def _():
        wait(fetch_group(1, 1))

    @head.append
    def _():
        _interleave(z_tasks(w3_first[0], 1), _merge(act_tasks(0), _singles(mac_tasks(0, 0)), _singles(kv_tasks(1))))
        _interleave(fwd_tasks(1))

    def transfers(s, p):
        f = s // NT
        wait(fetch_group(s + 1, 1 - p))
        start(fetch_group(jnp.minimum(s + 2, STEPS - 1), p))
        if p == 0:
            wait([fetch_w3(0)])
            start([fetch_w4(jnp.minimum(f + 1, NF - 1))])
        else:
            wait([fetch_w4(0)])
            start([fetch_w3(jnp.minimum(f + 2, NF - 1))])

    def step(s, p, row3, row4, row_out):
        if p == 0:
            w3c, w3_next = chunks(w3c_u, row3, W3_ROWS, 2)
            w4c, = chunks(w4c_u, row4, W4_ROWS, 1)
            prep = w3_combo_tasks(w3_next)
        else:
            w3c, = chunks(w3c_u, row3, W3_ROWS, 1)
            w4c, w4_next = chunks(w4c_u, row4, W4_ROWS, 2)
            prep = w4_combo_tasks(w4_next)
        first, second = z_tasks(w3c, 1 - p), w_tasks(w4c, 1 - p)
        inv, fwd = inv_tasks(row_out, 1 - p), fwd_tasks(1 - p)
        mo = cfg("mo", 4)
        if mo == 4: mxu, last = _merge(_singles(first), _singles(second), _singles(inv)), fwd
        if mo == 5: mxu, last = _merge(_singles(first[:-8]), _singles(second), _singles(inv)), fwd + first[-8:]
        if mo == 6: mxu, last = _merge(_singles(first), _singles(second), _singles(inv), _singles([fwd[1], fwd[3]])), [fwd[0], fwd[2]]
        if not cfg("prep", 1): prep = []
        act = act_tasks(p)
        if cfg("split", 0) == 1: act = [g for grp in act for g in (grp[:1], grp[1:])]
        if cfg("split", 0) == 2: act = [[x] for grp in act for x in grp]
        mac = _singles(mac_tasks(s, p)) if cfg("mac", 1) else []
        kvt = _singles(kv_tasks(1 - p)) if cfg("kv", 1) else []
        _interleave(mxu, _merge(act, mac, _singles(prep), kvt))
        _interleave(last)

    @tail_blocks.append
    def _():
        wait(fetch_group(STEPS - 1, 0) + [fetch_w4(NF - 1)])

    @tail_blocks.append
    def _():
        _interleave(w_tasks(w4_last, 0) + inv_tasks((STEPS - 2) * CG, 0), _merge(act_tasks(1), _singles(mac_tasks(STEPS - 1, 1))))

    @tail_blocks.append
    def _():
        _interleave(inv_tasks((STEPS - 1) * CG, 1) + w_tasks(w4_last, 1))

    @tail_blocks.append
    def _():
        _interleave(out_tasks(0, range(NB)))

    @tail_blocks.append
    def _():
        start(cp_o[:2])

    @tail_blocks.append
    def _():
        _interleave(out_tasks(1, range(NB)))

    @tail_blocks.append
    def _():
        start(cp_o[2:])
        wait(cp_o)

    region_ids = iter(range(100))

    def region(fn):
        with jax.named_scope("blk%d" % next(region_ids)):
            pl.when(pl.semaphore_read(idle) == 0)(fn)

    if cfg("head", 1):
        for fn in head:
            region(fn)

    def body(s, carry):
        rows = ((s + 1) // NT * (W3_ROWS // 2), (s - 1) // NT * (W4_ROWS // 2), (s - 1) * CG)
        pl.when(s % 2 == 1)(lambda: transfers(s, 1))
        pl.when(s % 2 == 0)(lambda: transfers(s, 0))
        with jax.named_scope("odd"):
            pl.when(s % 2 == 1)(lambda: step(s, 1, *rows))
        with jax.named_scope("even"):
            pl.when(s % 2 == 0)(lambda: step(s, 0, *rows))
        return carry

    if cfg("main", 1):
        lax.fori_loop(1, STEPS - 1, body, 0)
    if cfg("tail", 1):
        for fn in tail_blocks:
            region(fn)


@jax.jit
def pallas_gated_mix__ssm_conv_h3__mixer_s_mlp__prompt_kernel(
    A_q: jax.Array,
    A_k: jax.Array,
    A_v: jax.Array,
    A_shift_k: jax.Array,
    A_ssm_k: jax.Array,
    A_ssm_D: jax.Array,
    B_x: jax.Array,
    B_w1: jax.Array,
    B_w2: jax.Array,
    B_w3: jax.Array,
    B_w4: jax.Array,
    gate_w: jax.Array,
):
    del B_x
    vmem = pltpu.VMEM
    scratch = [
        vmem((D, S), bf16),
        vmem((D, D), bf16), vmem((D, D), bf16), vmem((D, FC), bf16), vmem((D, FC), bf16),
        vmem((KS, D), bf16), vmem((D,), bf16), vmem((D,), bf16), vmem((LANES, 2 * LANES), bf16),
        vmem((D, S), bf16),
        *[vmem((CG, S), bf16)] * 6, *[vmem((CG, (KS + 1) * LANES), f32)] * 2,
        vmem((D // 2, D), u32), vmem((D // 2, D), u32), vmem((LANES // 2, 2 * LANES), u32),
        vmem((D, (KS + 2) * LANES), f32), vmem((8, S), f32),
        vmem((D, S), f32), vmem((D // 2, S), u32), vmem((D // 2, S + 2 * LANES), u32),
        vmem((S, KM + LANES), f32),
        vmem((NT * NH * TS // 2, 2 * LANES), u32), vmem((S // 2, 2 * LANES), u32),
        vmem(((NF + 1) * W3_ROWS // 2, 2 * LANES), u32), vmem((NF * W4_ROWS // 2, 2 * LANES), u32),
        vmem((NT, NP, DS, TS), f32),
        vmem((NH * TS, 2 * LANES), f32), vmem((NH * TS, 2 * LANES), f32),
        vmem((NH * TS // 2, 2 * LANES), u32), vmem((NH * TS // 2, 2 * LANES), u32),
        vmem((NC * CG // 4, 2 * LANES), u32), vmem((NC * CG // 4, 2 * LANES), u32),
        vmem((NC * CG, 2 * LANES), f32), vmem((NC * CG, 2 * LANES), f32),
        vmem((NC * CG, 2 * LANES), f32), vmem((NC * CG, 2 * LANES), f32),
        vmem((NC * (CG + 32), 2 * LANES), f32), vmem((NC * (CG + 32), 2 * LANES), f32),
        vmem((D, S), f32),
        pltpu.SemaphoreType.DMA((32,)), pltpu.SemaphoreType.REGULAR,
    ]
    hbm = pl.BlockSpec(memory_space=pltpu.HBM)
    out_t = pl.pallas_call(
        _kernel,
        out_shape=jax.ShapeDtypeStruct((D, S), A_q.dtype),
        grid=(1,),
        in_specs=[hbm] * 12,
        out_specs=hbm,
        scratch_shapes=scratch,
        compiler_params=pltpu.CompilerParams(
            dimension_semantics=("arbitrary",), vmem_limit_bytes=124 * 2**20,
            flags={k: True for k in cfg("flags", "").split(",") if k} or None),
        name="gated_mix",
    )(A_q[0].T, A_k[0].T, A_v[0].T, A_shift_k.T, A_ssm_k, A_ssm_D, B_w1, B_w2, B_w3, B_w4.T,
      gate_w, _dft_matrix())
    return out_t.T[None]
```

```python
import functools
import math

import jax
import jax.numpy as jnp
import numpy as np
from jax import lax
from jax.experimental import pallas as pl
from jax.experimental.pallas import tpu as pltpu

S, D, F = 2048, 576, 4608
KS = 4
EPS = 1e-5
LANES = 128

NB, NP = 4, 49
NH = (NP + 1) // 2
FC = 512
NF = F // FC
TB = 1024
NT = S // TB
TS = TB // NB
KM = 512
KT = D - KM
KS3 = KM // NB
FS = FC // NB
DS = D // NB
STEPS = NF * NT
W4_ROWS = -(-NH * DS // 64) * 64
SKEW = 8

NC = S // LANES
CG = D // STEPS

GELU_C0 = math.sqrt(2.0 / math.pi)
GELU_C1 = GELU_C0 * 0.044715
GELU_S = GELU_C1 ** (1.0 / 3.0)

f32, bf16, u32 = jnp.float32, jnp.bfloat16, jnp.uint32
_NN = (((1,), (0,)), ((), ()))
_NT = (((1,), (1,)), ((), ()))

_AC = [{(0, 0): 1, (1, 1): 1}, {(1, 0): 1, (1, 1): 1}, {(0, 0): 1}, {(1, 1): 1},
       {(0, 0): 1, (0, 1): 1}, {(1, 0): 1, (0, 0): -1}, {(0, 1): 1, (1, 1): -1}]
_BC = [{(0, 0): 1, (1, 1): 1}, {(0, 0): 1}, {(0, 1): 1, (1, 1): -1}, {(1, 0): 1, (0, 0): -1},
       {(1, 1): 1}, {(0, 0): 1, (0, 1): 1}, {(1, 0): 1, (1, 1): 1}]
_CC = [{(0, 0): 1, (1, 1): 1}, {(1, 0): 1, (1, 1): -1}, {(0, 1): 1, (1, 1): 1},
       {(0, 0): 1, (1, 0): 1}, {(0, 0): -1, (0, 1): 1}, {(1, 1): 1}, {(0, 0): 1}]
_GATHER_ORDER = (0, 1, 2, 3, 5, 6, 4)
_TAIL = {6: (0, (0, 1)), 5: (1, (0, 1)), 1: (1, (0,)), 4: (0, (1,))}
_PAIRED = [(("s", 0), ("s", 0), ("s", 0), None, {(0, 0): 1, (1, 1): 1}),
           (("s", 0), ("s", 0), None, ("s", 0), {(0, 1): 1, (1, 0): 1}),
           (("s", 2), ("s", 3), ("s", 2), ("s", 3), {(0, 1): 1, (1, 1): 1}),
           (("s", 3), ("s", 2), ("s", 3), ("s", 2), {(0, 0): 1, (1, 0): 1}),
           (("s", 5), ("t", 1), ("s", 5), ("t", 1), {(1, 1): 1}),
           (("s", 6), ("t", 0), ("s", 6), ("t", 0), {(0, 0): 1}),
           (("t", 1), ("s", 5), ("t", 0), ("s", 5), {(1, 0): 1}),
           (("t", 0), ("s", 6), ("t", 1), ("s", 6), {(0, 1): 1}),
           (("s", 1), ("s", 1), ("s", 1), ("-", 1), {(1, 0): 1, (1, 1): -1}),
           (("s", 4), ("s", 4), ("s", 4), ("-", 4), {(0, 0): -1, (0, 1): 1})]
_PLAIN = [(("s", j), ("s", j), ("s", j), ("p", j), _CC[j]) for j in _GATHER_ORDER]
_INNER = [_PAIRED if i in _TAIL else _PLAIN for i in range(7)]
_FIRST = [sum(len(x) for x in _INNER[:i]) for i in range(8)]
NZ = _FIRST[7]
MIX = _PLAIN + _PAIRED
MIX_PAIRS = (len(MIX) + 1) // 2
ZH = (NZ + 1) // 2
W3_ROWS = ZH * KS3


def _dft_matrix():
    n = np.arange(LANES)[:, None]
    f = np.arange(LANES)[None, :]
    theta = np.pi * (((4 * f + 1) * n) % (4 * LANES)) / (2 * LANES)
    return np.concatenate([np.cos(theta), -np.sin(theta)], axis=1).astype(jnp.bfloat16)


def _mm(a, b, dims=_NN):
    return lax.dot_general(a, b, dims, preferred_element_type=f32)


def _gelu_scaled(y):
    return y * jnp.tanh(y * (y * y + GELU_C0 / GELU_S)) + y


def _combine(blocks, coef):
    n = len(blocks) // 2
    out = []
    for r in range(n):
        row = []
        for c in range(n):
            acc = None
            for (r0, c0), sign in coef.items():
                v = blocks[r0 * n + r][c0 * n + c]
                acc = v if acc is None else (acc + v if sign > 0 else acc - v)
            row.append(acc)
        out.append(row)
    return out


def _scatter(out, part, coef):
    n = len(part)
    for (r0, c0), sign in coef.items():
        for r in range(n):
            for c in range(n):
                o, v = out[r0 * n + r][c0 * n + c], part[r][c]
                out[r0 * n + r][c0 * n + c] = v if o is None else (o + v if sign > 0 else o - v)


def _gather_steps(get, out, inner=None):
    def one(i):
        part = [[None] * 2 for _ in range(2)]
        for j, spec in enumerate(inner[i] if inner else _PLAIN):
            _scatter(part, [[get(i, j)]], spec[-1])
        _scatter(out, part, _CC[i])
    return [functools.partial(one, i) for i in _GATHER_ORDER]


def _lhs_operands(blocks, tails, specs):
    def operand(kind, j):
        return tails[j] if kind == "t" else _combine(blocks, _AC[j])[0][0]
    out = []
    for low, high, *_ in specs:
        val = operand(*low)
        if high != low:
            val = jnp.concatenate([val[:, :KT], operand(*high)[:, KT:]], axis=1)
        out.append(val.astype(bf16))
    return out


def _rhs_operands(blocks, tails, specs, high):
    def operand(kind, j):
        if kind == "t":
            return tails[j]
        swap = high and kind != "p"
        val = _combine([row[::-1] for row in blocks] if swap else blocks, _BC[j])[0][0]
        return -val if kind == "-" else val
    picks = [spec[3 if high else 2] for spec in specs]
    return [(jnp.zeros_like(tails[0]) if pick is None else operand(*pick)).astype(bf16) for pick in picks]


def _weave(*streams):
    streams = [s for s in streams if s]
    total = [float(sum(w for w, _ in s)) for s in streams]
    pos, done, out = [0] * len(streams), [0.0] * len(streams), []
    while True:
        live = [k for k in range(len(streams)) if pos[k] < len(streams[k])]
        if not live:
            return out
        k = min(live, key=lambda j: (done[j] + 0.5 * streams[j][pos[j]][0]) / total[j])
        out.append(streams[k][pos[k]])
        done[k] += streams[k][pos[k]][0]
        pos[k] += 1


def _weave_groups(*streams):
    woven = _weave(*[[(sum(w for w, _ in grp), grp) for grp in s] for s in streams])
    return [t for _, grp in woven for t in grp]


def _run(tasks):
    for _, fn in tasks:
        fn()


def _kernel(q_hbm, k_hbm, v_hbm, shift_hbm, ssm_hbm, dd_hbm, w1_hbm, w2_hbm, w3_hbm, w4_hbm,
            gw_hbm, dft_hbm, o_hbm,
            q_u, w1_u, w2_u, w3_u, w4_u, shift_v, dd_v, gw_v, o_u,
            k_a, k_b, v_a, v_b, s_a, s_b, p_a, p_b, sh_a, sh_b,
            w1t_u, w2t_u, dft_u, w1c_u, w2c_u, pcol, gate, x1, xn_u, h1_u, xt_u, xc_u,
            w3c_u, w4c_u,
            acc, z_a, z_b, h_a, h_b, kv_a, kv_b, xf_a, xf_b, kf_a, kf_b, zf_a, zf_b,
            base, sems, idle):
    q_v, w1_v, w2_v, w3_v, w4_v, o_v, w1t, w2t, dft = (
        r.bitcast(bf16) for r in (q_u, w1_u, w2_u, w3_u, w4_u, o_u, w1t_u, w2t_u, dft_u))
    xn, h1, xt = (r.bitcast(bf16) for r in (xn_u, h1_u, xt_u))
    xc = [xc_u.at[pl.ds(t * ZH * TS // 2, ZH * TS // 2), :].bitcast(bf16) for t in range(NT)]
    z = (z_a, z_b)
    h = (h_a.bitcast(bf16), h_b.bitcast(bf16))
    kv = (kv_a.bitcast(bf16), kv_b.bitcast(bf16))
    xf, kf, mb = (xf_a, xf_b), (kf_a, kf_b), (zf_a, zf_b)
    kg, vg, sg = ([r.bitcast(bf16) for r in pair] for pair in ((k_a, k_b), (v_a, v_b), (s_a, s_b)))
    pg = (p_a, p_b)
    shifted = (sh_a, sh_b)
    task = functools.partial
    finished = set()

    def need(*tag):
        assert tag in finished, tag

    def rows_at(base, size, align):
        return pl.ds(base if isinstance(base, int) else pl.multiple_of(base, align), size)

    def tile(c):
        return pl.ds(c * LANES, LANES)

    def paired(i, height, offset, size):
        return pl.ds(i // 2 * height + offset, size), tile(i % 2)

    def product(i, offset, size):
        return paired(i, TS, offset, size)

    def chunks(ref_u32, first_row, rows, count):
        window = ref_u32.at[rows_at(first_row, count * (rows // 2), 8), :]
        return [window.at[pl.ds(i * (rows // 2), rows // 2), :].bitcast(bf16) for i in range(count)]

    sem_ids = iter(range(sems.shape[0]))

    def copy(src, dst):
        return pltpu.make_async_copy(src, dst, sems.at[next(sem_ids)])

    cp_q = [copy(q_hbm.at[:, pl.ds(a, b - a)], q_v.at[:, pl.ds(a, b - a)])
            for a, b in ((0, 2 * LANES), (2 * LANES, 4 * LANES), (4 * LANES, 8 * LANES), (8 * LANES, 12 * LANES), (12 * LANES, S))]
    cp_w1, cp_w2 = copy(w1_hbm, w1_v), copy(w2_hbm, w2_v)
    cp_gate, cp_small = copy(gw_hbm, gw_v), [copy(shift_hbm, shift_v), copy(dd_hbm, dd_v), copy(dft_hbm, dft)]
    sem_w3, sem_w4 = (sems.at[next(sem_ids)] for _ in range(2))
    sem_conv = [[sems.at[next(sem_ids)] for _ in range(5)] for _ in range(2)]
    def put(t, c, r0, r1):
        cols = pl.ds(t * TB + c * NB * LANES, NB * LANES)
        bands = [pl.ds(0, D)] if r1 - r0 == DS else [pl.ds(a * DS + r0, r1 - r0) for a in range(NB)]
        return [copy(o_v.at[rows, cols], o_hbm.at[rows, cols]) for rows in bands]

    def fetch_w3(f):
        return pltpu.make_async_copy(w3_hbm.at[:, rows_at(f * FC, FC, FC)], w3_v, sem_w3)

    def fetch_w4(f):
        return pltpu.make_async_copy(w4_hbm.at[:, rows_at(f * FC, FC, FC)], w4_v, sem_w4)

    def fetches(s, p):
        def rows(g):
            return rows_at(g * CG, CG, CG)

        cps = []
        for ahead, pairs in ((4, [(k_hbm, 0, kg)]), (3, [(v_hbm, 0, vg), (pcol, 0, pg)]), (2, [(ssm_hbm, 0, sg)])):
            g, slot = s + ahead, (p + ahead) % 2
            if isinstance(g, int):
                if not 0 <= g < STEPS:
                    continue
            for src, col, dst in pairs:
                if not isinstance(g, int):
                    top = STEPS if src is pcol else STEPS - 1
                    at = jnp.minimum(g, top)
                else:
                    at = g
                sem = sem_conv[p][len(cps)]
                cps.append(pltpu.make_async_copy(
                    src.at[rows(at), pl.ds(col, dst[slot].shape[1])], dst[slot], sem))
        return cps

    def start(cps):
        for cp in cps:
            cp.start()

    def wait(cps):
        for cp in cps:
            cp.wait()

    def transpose_tasks(src, dst):
        def t(c0, c1):
            dst[c0:c1, :] = jnp.concatenate([src[:, c0:c1], src[KM:D, c0:c1]], axis=0).T
        return [(1, task(t, c0, min(D, c0 + LANES))) for c0 in range(0, D, LANES)]

    def param_tasks():
        def column(j):
            row = (shift_v[j:j + 1, :].astype(f32) if j < KS
                   else (dd_v, gw_v)[j - KS][...].astype(f32).reshape(1, D))
            top = CG if j == KS else 0
            pcol[pl.ds(top, D), tile(j)] = jnp.broadcast_to(row, (LANES, D)).T
            pcol[pl.ds(D - D * (j == KS), CG), tile(j)] = jnp.zeros((CG, LANES), f32)

        def pad():
            zero = jnp.zeros((D // 2, LANES), u32)
            h1_u[:, 0:LANES] = zero
            h1_u[:, LANES + S:] = zero
        return [(1, task(column, KS + 1)), (1, pad)] + [(1, task(column, j)) for j in range(KS + 1)]

    RG = 48
    NG = D // RG

    def fold(x):
        return functools.reduce(lambda u, v: u + v, [x[i:i + 8] for i in range(0, RG, 8)])

    def norm_tasks(c, load, emit):
        st = {"sum": 0.0, "sq": 0.0}

        def sweep1(g):
            st["sum"] = st["sum"] + fold(load(g, True))
            if g == NG - 1:
                st["mean"] = jnp.sum(st["sum"], axis=0, keepdims=True) * (1.0 / D)

        def sweep2(g):
            d = load(g, False) - st["mean"]
            st["sq"] = st["sq"] + fold(d * d)
            if g == NG - 1:
                var = jnp.sum(st["sq"], axis=0, keepdims=True) * (1.0 / D)
                st["rstd"] = lax.rsqrt(var + EPS) * GELU_S

        def sweep3(g):
            emit(g, ((load(g, False) - st["mean"]) * st["rstd"]).astype(bf16))
        return [[(20, task(fn, g)) for g in range(NG)] for fn in (sweep1, sweep2, sweep3)]

    def ln0_tasks(c):
        st = {"logit": 0.0}

        def load(g, first):
            rs = pl.ds(g * RG, RG)
            if not first:
                return x1[rs, tile(c)]
            x = q_v[rs, tile(c)].astype(f32)
            x1[rs, tile(c)] = x
            st["logit"] = st["logit"] + fold(x * pcol[rs, tile(KS + 1)])
            if g == NG - 1:
                logit = jnp.sum(st["logit"], axis=0, keepdims=True)
                gate[:, tile(c)] = jnp.broadcast_to(jax.nn.sigmoid(logit), (8, LANES))
            return x

        def emit(g, val):
            xn[pl.ds(g * RG, RG), tile(c)] = val
            finished.add(("xn", c, g))
        return norm_tasks(c, load, emit)

    def ln1_tasks(c):
        def emit(g, val):
            xn[pl.ds(g * RG, RG), tile(c)] = val
        def load(g, first):
            need("x1", c, g * RG)
            return x1[pl.ds(g * RG, RG), tile(c)]
        return norm_tasks(c, load, emit)

    def to_token_major(c):
        def t():
            tail = xn[KM:D, tile(c)]
            xt[tile(c), :] = jnp.concatenate([xn[:, tile(c)], tail], axis=0).T
        return [(1, t)]

    def mix_tasks(wt, finish, tiles):
        ts, pending = [], []
        for c in tiles:
            for g in range(NB):
                st = {}

                def one(k, c=c, g=g, st=st):
                    k0, k1 = k * LANES, min(D, (k + 1) * LANES)
                    y = _mm(wt[pl.ds(g * DS, DS), k0:k1], xn[k0:k1, tile(c)])
                    st["y"] = y if k == 0 else st["y"] + y
                for k in range(pl.cdiv(D, LANES)):
                    ts.append((DS, task(one, k)))
                    if pending:
                        ts.append((0, pending.pop(0)))
                pending = [task(lambda c, row, st, r: finish(c, row, st["y"][r:r + RG]), c, g * DS + r, st, r)
                           for r in range(0, DS, RG)]
        return ts + [(0, fn) for fn in pending]

    def mix_rhs(pair):
        rows = MIX_PAIRS * LANES
        return (h_a, h_b)[pair % 2].at[pl.ds(pair // 2 * rows // 2, rows // 2), :].bitcast(bf16)

    def mix_lhs_groups(wt, dst):
        dst, half = dst.bitcast(bf16), D // 2

        def t(r, part):
            blk = [[wt[pl.ds(a * half + r, 16), tile(2 * k + part)].astype(f32) for k in range(2)] for a in range(2)]
            tails = [wt[pl.ds(a * half + r, 16), tile(NB)].astype(f32) for a in range(2)]
            for n, val in enumerate(_lhs_operands(blk, tails, (_PLAIN, _PAIRED)[part])):
                dst[paired(part * len(_PLAIN) + n, half, r, 16)] = val
        return [[(40, task(t, r, part))] for r in range(0, half, 16) for part in range(2)]

    def mix_rhs_groups(pair):
        dst = mix_rhs(pair)

        def t(r, part):
            need("xn", 2 * pair + 1, NG - 1)
            blk = [[xn[pl.ds((2 * k + part) * LANES + r, 16), tile(2 * pair + b)].astype(f32)
                    for b in range(2)] for k in range(2)]
            tails = [xn[pl.ds(KM + r % KT, 16), tile(2 * pair + b)].astype(f32) for b in range(2)]
            for n, val in enumerate(_rhs_operands(blk, tails, (_PLAIN, _PAIRED)[part], r >= KT)):
                dst[paired(part * len(_PLAIN) + n, LANES, r, 16)] = val
        return [[(40, task(t, r, part))] for r in range(0, LANES, 16) for part in range(2)]

    def fast_mix_tasks(wc, finish, pairs):
        wc, half = wc.bitcast(bf16), D // 2
        ts, pending = [], []
        for pair in pairs:
            for r in range(0, half, RG):
                out = [[None] * 2 for _ in range(2)]

                def one(n, pair=pair, r=r, out=out):
                    y = _mm(wc[paired(n, half, r, RG)], mix_rhs(pair)[paired(n, LANES, 0, LANES)])
                    _scatter(out, [[y]], MIX[n][-1])
                for n in range(len(MIX)):
                    ts.append((RG, task(one, n)))
                    if pending and n % 2:
                        ts.append((0, pending.pop(0)))
                pending = [task(lambda a, b, r, out, pair: finish(2 * pair + b, a * half + r, out[a][b]), a, b, r, out, pair)
                           for a in range(2) for b in range(2)]
        return ts + [(0, fn) for fn in pending]

    def h1_finish(c, row, y):
        h1[pl.ds(row, RG), tile(c + 1)] = ((0.5 / GELU_S) * _gelu_scaled(y)).astype(bf16)

    def spatial_shift(c):
        rows = D // 8

        def t(g, shift):
            rs = pl.ds(g * rows, rows)
            xn_u[rs, tile(c)] = h1_u[rs, pl.ds((c + 1) * LANES - shift, LANES)]
        return [(1, task(t, g, shift)) for g, shift in enumerate((1, -1, 2, -2))]

    def hs_finish(c, row, y):
        x1[pl.ds(row, RG), tile(c)] += y
        finished.add(("x1", c, row))

    def each(fn, tiles):
        return [t for c in tiles for t in fn(c)]

    def combo_group(load, coef, store):
        blk = [[None] * NB for _ in range(NB)]

        def fetch(a):
            blk[a][:] = [load(a, b) for b in range(NB)]

        def emit(i):
            mid = _combine(blk, coef[i])
            for j in range(7):
                store(7 * i + j, _combine(mid, coef[j])[0][0].astype(bf16))
        return [(20, task(fetch, a)) for a in range(NB)] + [(32, task(emit, i)) for i in range(7)]

    def token(t, b, offset):
        return t * TB + (offset // LANES * NB + b) * LANES + offset % LANES

    def xc_groups(t):
        out = []
        for r in range(TS // 16):
            blk, tails = [[None] * NB for _ in range(NB)], [None] * NB

            def fetch(b, r=r, blk=blk, tails=tails):
                rs = pl.ds(token(t, b, r * 16), 16)
                blk[b][:] = [xt[rs, tile(k)].astype(f32) for k in range(NB)]
                tails[b] = xt[rs, tile(NB)].astype(f32)

            def emit(i, r=r, blk=blk, tails=tails):
                row = 2 * _TAIL[i][0] if i in _TAIL else 0
                for n, val in enumerate(_lhs_operands(_combine(blk, _AC[i]), tails[row:row + 2], _INNER[i])):
                    xc[t][product(_FIRST[i] + n, r * 16, 16)] = val
            out.append([(22, task(fetch, b)) for b in range(NB)]
                       + [(5 * len(_INNER[i]), task(emit, i)) for i in range(7)])
        return out

    def w3_groups(dst):
        out = []
        for r in range(KS3 // 16):
            high = r >= KT // 16
            blk, tails = [[None] * NB for _ in range(NB)], [None] * NB

            def fetch(k, r=r, blk=blk, tails=tails):
                blk[k][:] = [w3_v[pl.ds(k * KS3 + r * 16, 16), tile(a)].astype(f32) for a in range(NB)]
                tails[k] = w3_v[pl.ds(KM + r * 16 % KT, 16), tile(k)].astype(f32)

            def emit(i, r=r, high=high, blk=blk, tails=tails):
                cols = _TAIL[i][1] if i in _TAIL else (0,)
                sums = [functools.reduce(lambda x, y: x + y, [tails[2 * u + j] for u in cols]) for j in range(2)]
                for n, val in enumerate(_rhs_operands(_combine(blk, _BC[i]), sums, _INNER[i], high)):
                    dst[paired(_FIRST[i] + n, KS3, r * 16, 16)] = val
            out.append([(16, task(fetch, k)) for k in range(NB)]
                       + [(5 * len(_INNER[i]), task(emit, i)) for i in range(7)])
        return out

    def w4_groups(dst):
        out = []
        for r in range(DS // 16):
            def store(i, val, r=r):
                dst[paired(i, DS, r * 16, 16)] = val
            out.append(combo_group(
                lambda a, b, r=r: w4_v[pl.ds(a * DS + r * 16, 16), tile(b)].astype(f32), _AC, store))
        return out

    def clear_tasks(lo, hi):
        def t(n):
            acc[n // NP, n % NP] = jnp.zeros((DS, TS), f32)
        return [(36, task(t, n)) for n in range(lo, hi)]

    def copy_clear_groups(lo, hi):
        def t(n, r):
            acc[n // NP, n % NP, pl.ds(r, RG)] = acc[(n - 1) // NP, (n - 1) % NP, pl.ds(r, RG)]
        return [[(12, task(t, n, r))] for n in range(lo, hi) for r in range(0, DS, RG)]

    def z_tasks(w3c, t):
        m = TS // 4

        def prod(i, r0):
            z[t][product(i, r0, m)] = _mm(xc[t][product(i, r0, m)], w3c[paired(i, KS3, 0, KS3)])
        return [(m, task(prod, i, r0)) for i in range(NZ) for r0 in range(0, TS, m)]

    def act_groups(t):
        out = []
        for r in range(TS // 16):
            grp, halves = [], []
            for r0 in (r * 16, r * 16 + 8):
                pre = [[None] * NB for _ in range(NB)]
                act = [[None] * NB for _ in range(NB)]
                grp += [(24, fn) for fn in _gather_steps(
                    lambda i, j, r0=r0: z[t][product(_FIRST[i] + j, r0, 8)], pre, _INNER)]

                def activate(a, pre=pre, act=act):
                    act[a][:] = [_gelu_scaled(pre[b][a]) for b in range(NB)]
                grp += [(30, task(activate, a)) for a in range(NB)]
                halves.append(act)

            def emit(i, r=r, halves=halves):
                lo, hi = _combine(halves[0], _BC[i]), _combine(halves[1], _BC[i])
                for j in range(7):
                    v = jnp.concatenate([_combine(lo, _BC[j])[0][0], _combine(hi, _BC[j])[0][0]], axis=0)
                    h[t][product(7 * i + j, r * 16, 16)] = v.astype(bf16)
            out.append(grp + [(40, task(emit, i)) for i in range(7)])
        return out

    def w_tasks(w4c, t, by_tile=False):
        def prod(i, c):
            acc[t, i, :, tile(c)] += _mm(w4c[paired(i, DS, 0, DS)], h[t][product(i, c * LANES, LANES)], _NT)
        tiles = range(TS // LANES)
        order = [(i, c) for c in tiles for i in range(NP)] if by_tile else [(i, c) for i in range(NP) for c in tiles]
        return [(DS, task(prod, i, c)) for i, c in order]

    def shift_tasks(p):
        def t(j):
            words = (k_a, k_b)[p][...]
            if j:
                words = pltpu.roll(words, j, axis=1)
                lane = lax.broadcasted_iota(jnp.int32, (CG // 2, LANES), 1)
                shifted[p][pl.ds(j * CG // 2, CG // 2), tile(0)] = jnp.where(lane >= j, words[:, :LANES], 0)
                shifted[p][pl.ds(j * CG // 2, CG // 2), LANES:] = words[:, LANES:]
            else:
                shifted[p][0:CG // 2, :] = words
        return [(1, task(t, j)) for j in range(KS)]

    def kv_groups(p):
        delayed = shifted[p].bitcast(bf16)

        def t(c, r):
            rs = pl.ds(r * 16, 16)
            ksum = None
            for j in range(KS):
                term = delayed[pl.ds(j * CG + r * 16, 16), tile(c)].astype(f32) * pg[p][rs, tile(j)]
                ksum = term if ksum is None else ksum + term
            kv[p][pl.ds(c % (NC // 2) * CG + r * 16, 16), tile(c // (NC // 2))] = (
                ksum * vg[p][rs, tile(c)].astype(f32)).astype(bf16)
        n = 2
        return [[(36, task(t, c, r)) for c in range(c0, c0 + n)] for r in range(CG // 16) for c0 in range(0, NC, n)]

    HALF = NC // 2 * CG

    def data_dft_tasks(p):
        m = HALF // 4

        def t(part, c, r0):
            xf[p][pl.ds(part * HALF + r0, m), tile(c)] = _mm(kv[p][pl.ds(r0, m), tile(part)], dft[:, tile(c)])
        return [(m, task(t, part, c, r0)) for part in range(2) for c in range(2) for r0 in range(0, HALF, m)]

    def filter_dft_tasks(p):
        n = NC // 2 // 4

        def t(j0, c):
            lhs = jnp.concatenate([sg[p][:, tile(j)] for j in range(j0, j0 + n)], axis=0)
            y = _mm(lhs, dft[:, tile(c)])
            if j0 == 0 and c == 0:
                kf[p][0:CG, tile(0)] = y[0:CG] + pg[1 - p][:, tile(KS)]
                kf[p][CG:n * CG, tile(0)] = y[CG:]
            else:
                kf[p][pl.ds(j0 * CG, n * CG), tile(c)] = y
        return [(n * CG, task(t, j0, c)) for j0 in range(0, NC, n) for c in range(2)]

    def mac_groups(p):
        out = []
        block_size = 2
        for u in range(CG // 8):
            full = {}

            def spectrum(ref, j, u=u):
                rs = pl.ds(j * CG + u * 8, 8)
                return ref[rs, tile(0)], ref[rs, tile(1)]

            for i0 in range(0, NC, block_size):
                data = {}

                def add(m, i0=i0, spectrum=spectrum, full=full, data=data):
                    c, d = spectrum(kf[p], m)
                    for i in range(max(i0, m), i0 + block_size):
                        if i - m not in data:
                            data[i - m] = spectrum(xf[p], i - m)
                        a, b = data[i - m]
                        if i in full:
                            full[i] = (full[i][0] + a * c - b * d, full[i][1] + a * d + b * c)
                        else:
                            full[i] = (a * c - b * d, a * d + b * c)

                def finish(i0=i0, u=u, full=full):
                    for i in range(i0, i0 + block_size):
                        re, im = full[i]
                        if i:
                            re, im = re - full[i - 1][1], im + full[i - 1][0]
                        mb[p][pl.ds(i * CG + u * 8, 8), tile(0)] = re
                        mb[p][pl.ds(i * CG + u * 8, 8), tile(1)] = im
                top = i0 + block_size
                out.append([(4 + 8 * (top - max(i0, m)), task(add, m)) for m in range(top)]
                           + [(4 * block_size, finish)])
        return out

    def inverse_dft_tasks(row, p):
        qg, xg, og = (ref.at[rows_at(row, CG, CG), :] for ref in (q_v, x1, base))
        n = 4
        rows = NC * CG // n

        def t(part):
            y = _mm(mb[p][pl.ds(part * rows, rows), :].astype(bf16), dft[...], _NT)
            for j in range(NC // n):
                cs = tile(part * NC // n + j)
                g = jnp.concatenate([gate[:, cs]] * (CG // 8), axis=0)
                conv = y[j * CG:(j + 1) * CG] * qg[:, cs].astype(f32)
                og[:, cs] = (g * (1.0 / LANES)) * conv + (1.0 - g) * xg[:, cs]
        return [(2 * rows, task(t, part)) for part in range(n)]

    def conv_stage(s, p, row, products):
        def live(g):
            return not isinstance(g, int) or 0 <= g < STEPS
        mxu, vpu, xlu = [], [], []
        if live(s):
            mxu.append(inverse_dft_tasks(row, p))
        if live(s + 1) and products:
            vpu.append(mac_groups(1 - p))
        if live(s + 2):
            mxu += [filter_dft_tasks(p), data_dft_tasks(p)]
        if live(s + 3):
            vpu.append(kv_groups(1 - p))
        if live(s + 4):
            xlu = shift_tasks(p)
        return mxu, vpu, xlu

    def out_groups(t, c, r0, r1):
        out = []
        for row in range(r0, r1, 16):
            grp, halves = [], []
            for top in (row, row + 8):
                blk = [[None] * NB for _ in range(NB)]
                grp += [(24, fn) for fn in _gather_steps(
                    lambda i, j, top=top: acc[t, 7 * i + _GATHER_ORDER[j], pl.ds(top, 8), tile(c)], blk)]

                def mix(b, top=top, blk=blk):
                    tok = pl.ds(token(t, b, c * LANES), LANES)
                    scale = (1.0 - gate[:, tok]) * (0.5 / GELU_S)
                    for a in range(NB):
                        blk[a][b] = base[pl.ds(a * DS + top, 8), tok] + scale * blk[a][b]
                grp += [(15, task(mix, b)) for b in range(NB)]
                halves.append(blk)

            def put_rows(b, row=row, halves=halves):
                tok = pl.ds(token(t, b, c * LANES), LANES)
                for a in range(NB):
                    o_v[pl.ds(a * DS + row, 16), tok] = jnp.concatenate(
                        [halves[0][a][b], halves[1][a][b]], axis=0).astype(bf16)
            out.append(grp + [(8, task(put_rows, b)) for b in range(NB)])
        return out

    def block(fn):
        pl.when(pl.semaphore_read(idle) == 0)(fn)

    def compute(mxu=(), vpu=(), xlu=()):
        _run(_weave(_weave(*mxu), _weave_groups(*vpu)) + list(xlu))

    def staggered(fn, tiles):
        sweeps = [fn(c) for c in tiles]
        return [_weave(*[sweeps[i - k][k] for k in range(3) if 0 <= i - k < len(sweeps)])
                for i in range(len(sweeps) + 2)]

    def exchange(done, begin):
        wait(done)
        start(begin)

    def inputs(s, p):
        fetch = (fetch_w3, fetch_w4)[p]
        if isinstance(s, int):
            return fetches(s, p) + ([fetch(s // NT + 1)] if s > 0 else [])
        return fetches(s, p) + [fetch(jnp.minimum(s // NT + 1, NF - 1))]

    def stage(s, p, row, mxu=(), vpu=(), xlu=(), products=True):
        m, v, x = conv_stage(s, p, row, products)
        compute(list(mxu) + m, list(vpu) + v, list(xlu) + x)

    def fixed_stage(s, mxu=(), vpu=(), xlu=(), also=(), products=True):
        exchange(inputs(s, s % 2) + list(also), inputs(s + 1, 1 - s % 2))
        block(lambda: stage(s, s % 2, s * CG, mxu, vpu, xlu, products))

    def step(s, p, row3, row4, row_out):
        if p == 0:
            w3c, w3_next = chunks(w3c_u, row3, W3_ROWS, 2)
            w4c, = chunks(w4c_u, row4, W4_ROWS, 1)
            prep = w3_groups(w3_next)
        else:
            w3c, = chunks(w3c_u, row3, W3_ROWS, 1)
            w4c, w4_next = chunks(w4c_u, row4, W4_ROWS, 2)
            prep = w4_groups(w4_next)
        stage(s, p, row_out, [z_tasks(w3c, 1 - p), w_tasks(w4c, 1 - p)], [act_groups(p), prep])

    def step_rows(s):
        return (s + 1) // NT * (W3_ROWS // 2) + SKEW, (s - 1) // NT * (W4_ROWS // 2) + SKEW, s * CG

    def chunk(ref_u32, f, rows):
        return chunks(ref_u32, f * (rows // 2) + SKEW, rows, 1)[0]

    start([cp_gate, cp_q[0], cp_w1, cp_q[1]] + cp_small + cp_q[2:] + [cp_w2, fetch_w3(0), fetch_w4(0)])
    c1, c2, c3 = 28, 64, 10
    block(lambda: compute([], [[clear_tasks(0, c1)]]))
    exchange([cp_gate], [])
    block(lambda: compute([], [], param_tasks()[:2]))
    exchange([cp_q[0]], [])
    block(lambda: compute([], [staggered(ln0_tasks, range(2))]))
    block(lambda: compute([], [[clear_tasks(c1, c2)]]))
    exchange([cp_w1], [])
    block(lambda: compute([], [], transpose_tasks(w1_v, w1t)))

    def first(pairs):
        return fast_mix_tasks(w1c_u, h1_finish, pairs)

    def second(pairs):
        return fast_mix_tasks(w2c_u, hs_finish, pairs)

    def operands(pairs):
        return [grp for pair in pairs for grp in mix_rhs_groups(pair)]

    block(lambda: compute([mix_tasks(w1t, h1_finish, [0])], [mix_lhs_groups(w1t, w1c_u)]))
    exchange([cp_q[1]], [])
    block(lambda: compute([mix_tasks(w1t, h1_finish, [1])], [staggered(ln0_tasks, range(2, 4)) + operands([1])]))
    exchange([cp_q[2]] + cp_small, [])
    block(lambda: compute([first([1])], [staggered(ln0_tasks, range(4, 8)) + operands([2, 3])]))
    exchange([cp_q[3]], inputs(-4, 0))
    block(lambda: compute([first([2, 3])], [staggered(ln0_tasks, range(8, 12)) + operands([4, 5]), copy_clear_groups(c2, c2 + c3)]))
    exchange([cp_q[4], cp_w2], [])
    block(lambda: compute([first([4, 5])], [staggered(ln0_tasks, range(12, NC)) + operands([6, 7]), copy_clear_groups(c2 + c3, c2 + 2 * c3)],
                          transpose_tasks(w2_v, w2t) + each(spatial_shift, range(6))))
    block(lambda: compute([first([6, 7])],
                          [mix_lhs_groups(w2t, w2c_u), operands([0, 1, 2])],
                          each(spatial_shift, range(6, 10))))
    exchange([fetch_w3(0), fetch_w4(0)], [])
    block(lambda: compute([second([0, 1, 2])],
                          [operands([3, 4]), w3_groups(chunk(w3c_u, 0, W3_ROWS)) + w4_groups(chunk(w4c_u, 0, W4_ROWS)),
                           copy_clear_groups(c2 + 2 * c3, NT * NP)],
                          each(spatial_shift, range(10, NC))))
    exchange([], [fetch_w3(1)])
    block(lambda: compute([second([3, 4])], [operands([5, 6, 7]), staggered(ln1_tasks, range(8))], param_tasks()[2:]))
    fixed_stage(-4, [second([5])], [staggered(ln1_tasks, range(8, 10))],
                each(to_token_major, range(8)))
    fixed_stage(-3, [second([6, 7])], [staggered(ln1_tasks, range(10, 12)), xc_groups(0)])
    z_first = z_tasks(chunk(w3c_u, 0, W3_ROWS), 0)
    cut = len(z_first) * 24 // 100
    cut1 = len(z_first) * 68 // 100
    fixed_stage(-2, [z_first[:cut]], [staggered(ln1_tasks, range(12, NC))], each(to_token_major, range(8, 12)),
                also=[fetch_w3(1)])
    block(lambda: compute([z_first[cut:cut1]], [w3_groups(chunk(w3c_u, 1, W3_ROWS)), mac_groups(0)],
                          each(to_token_major, range(12, NC))))
    fixed_stage(-1, [z_first[cut1:]], [xc_groups(1)], products=False)
    fixed_stage(0, [z_tasks(chunk(w3c_u, 0, W3_ROWS), 1)], [act_groups(0)])

    def body(i, carry):
        for p in (1, 0):
            s = 2 * i + 2 - p
            rows = step_rows(s)
            exchange(inputs(s, p), inputs(s + 1, 1 - p))
            block(task(step, s, p, *rows))
        return carry

    last = STEPS - 2
    lax.fori_loop(0, last // 2, body, 0)

    exchange(inputs(jnp.int32(last + 1), 1), [])
    w4_last = chunk(w4c_u, NF - 1 + pl.semaphore_read(idle), W4_ROWS)
    block(lambda: stage(last + 1, 1, (last + 1) * CG, [w_tasks(w4_last, 0)], [act_groups(1)]))
    w_last = w_tasks(w4_last, 1, by_tile=True)
    pieces = [(0, 0, 0, DS), (0, 1, 0, DS), (1, 0, 0, DS), None, (1, 1, 0, 80), (1, 1, 80, DS)]
    cuts = [0, 26, 52, NP + 30, 2 * NP, 2 * NP, 2 * NP]
    sent = []
    for n, piece in enumerate(pieces):
        span = w_last[cuts[n]:cuts[n + 1]]
        block(lambda: compute([span], [out_groups(*piece)] if piece else []))
        if piece:
            sent += put(*piece)
            exchange([], sent[-(1 if piece[3] - piece[2] == DS else NB):])
    wait(sent)


@jax.jit
def pallas_gated_mix__ssm_conv_h3__mixer_s_mlp__prompt_kernel(
    A_q: jax.Array,
    A_k: jax.Array,
    A_v: jax.Array,
    A_shift_k: jax.Array,
    A_ssm_k: jax.Array,
    A_ssm_D: jax.Array,
    B_x: jax.Array,
    B_w1: jax.Array,
    B_w2: jax.Array,
    B_w3: jax.Array,
    B_w4: jax.Array,
    gate_w: jax.Array,
):
    del B_x
    vmem = pltpu.VMEM
    scratch = [
        vmem((D // 2, S), u32),
        *[vmem((D // 2, D), u32)] * 2, *[vmem((D // 2, FC), u32)] * 2,
        vmem((KS, D), bf16), vmem((D,), bf16), vmem((D,), bf16),
        vmem((D // 2, S), u32),
        *[vmem((CG // 2, S), u32)] * 6, *[vmem((CG, (KS + 1) * LANES), f32)] * 2,
        *[vmem((KS * CG // 2, S), u32)] * 2,
        *[vmem((D // 2, KM + LANES), u32)] * 2, vmem((LANES // 2, 2 * LANES), u32),
        *[vmem((MIX_PAIRS * D // 4, 2 * LANES), u32)] * 2,
        vmem((D + CG, (KS + 2) * LANES), f32), vmem((8, S), f32),
        vmem((D, S), f32), vmem((D // 2, S), u32), vmem((D // 2, S + 2 * LANES), u32),
        vmem((S // 2, KM + LANES), u32),
        vmem((NT * ZH * TS // 2, 2 * LANES), u32),
        vmem(((NF + 1) * W3_ROWS // 2 + 32, 2 * LANES), u32), vmem((NF * W4_ROWS // 2 + 32, 2 * LANES), u32),
        vmem((NT, NP, DS, TS), f32),
        vmem((ZH * TS, 2 * LANES), f32), vmem((ZH * TS, 2 * LANES), f32),
        vmem((NH * TS // 2, 2 * LANES), u32), vmem((NH * TS // 2, 2 * LANES), u32),
        vmem((NC * CG // 4, 2 * LANES), u32), vmem((NC * CG // 4, 2 * LANES), u32),
        vmem((NC * CG, 2 * LANES), f32), vmem((NC * CG, 2 * LANES), f32),
        vmem((NC * CG, 2 * LANES), f32), vmem((NC * CG, 2 * LANES), f32),
        vmem((NC * CG, 2 * LANES), f32), vmem((NC * CG, 2 * LANES), f32),
        vmem((D, S), f32),
        pltpu.SemaphoreType.DMA((40,)), pltpu.SemaphoreType.REGULAR,
    ]
    hbm = pl.BlockSpec(memory_space=pltpu.HBM)
    out_t = pl.pallas_call(
        _kernel,
        out_shape=jax.ShapeDtypeStruct((D, S), A_q.dtype),
        grid=(1,),
        in_specs=[hbm] * 12,
        out_specs=hbm,
        scratch_shapes=scratch,
        compiler_params=pltpu.CompilerParams(
            dimension_semantics=("arbitrary",), vmem_limit_bytes=124 * 2**20,
            disable_bounds_checks=bool(1)),
        name="gated_mix",
    )(A_q[0].T, A_k[0].T, A_v[0].T, A_shift_k.T, A_ssm_k, A_ssm_D, B_w1, B_w2, B_w3, B_w4.T,
      gate_w, _dft_matrix())
    return out_t.T[None]
```

```python
import functools
import math

import jax
import jax.numpy as jnp
import numpy as np
from jax import lax
from jax.experimental import pallas as pl
from jax.experimental.pallas import tpu as pltpu

S, D, F = 2048, 576, 4608
KS = 4
EPS = 1e-5
LANES = 128

NB, NP = 4, 49
NH = (NP + 1) // 2
FC = 512
NF = F // FC
TB = 1024
NT = S // TB
TS = TB // NB
KM = 512
KT = D - KM
KS3 = KM // NB
FS = FC // NB
DS = D // NB
STEPS = NF * NT
W4_ROWS = -(-NH * DS // 64) * 64
SKEW = 8

NC = S // LANES
CG = D // STEPS

GELU_C0 = math.sqrt(2.0 / math.pi)
GELU_C1 = GELU_C0 * 0.044715
GELU_S = GELU_C1 ** (1.0 / 3.0)

f32, bf16, u32 = jnp.float32, jnp.bfloat16, jnp.uint32
_NN = (((1,), (0,)), ((), ()))
_NT = (((1,), (1,)), ((), ()))

_AC = [{(0, 0): 1, (1, 1): 1}, {(1, 0): 1, (1, 1): 1}, {(0, 0): 1}, {(1, 1): 1},
       {(0, 0): 1, (0, 1): 1}, {(1, 0): 1, (0, 0): -1}, {(0, 1): 1, (1, 1): -1}]
_BC = [{(0, 0): 1, (1, 1): 1}, {(0, 0): 1}, {(0, 1): 1, (1, 1): -1}, {(1, 0): 1, (0, 0): -1},
       {(1, 1): 1}, {(0, 0): 1, (0, 1): 1}, {(1, 0): 1, (1, 1): 1}]
_CC = [{(0, 0): 1, (1, 1): 1}, {(1, 0): 1, (1, 1): -1}, {(0, 1): 1, (1, 1): 1},
       {(0, 0): 1, (1, 0): 1}, {(0, 0): -1, (0, 1): 1}, {(1, 1): 1}, {(0, 0): 1}]
_GATHER_ORDER = (0, 1, 2, 3, 5, 6, 4)
_TAIL = {6: (0, (0, 1)), 5: (1, (0, 1)), 1: (1, (0,)), 4: (0, (1,))}
_PAIRED = [(("s", 0), ("s", 0), ("s", 0), None, {(0, 0): 1, (1, 1): 1}),
           (("s", 0), ("s", 0), None, ("s", 0), {(0, 1): 1, (1, 0): 1}),
           (("s", 2), ("s", 3), ("s", 2), ("s", 3), {(0, 1): 1, (1, 1): 1}),
           (("s", 3), ("s", 2), ("s", 3), ("s", 2), {(0, 0): 1, (1, 0): 1}),
           (("s", 5), ("t", 1), ("s", 5), ("t", 1), {(1, 1): 1}),
           (("s", 6), ("t", 0), ("s", 6), ("t", 0), {(0, 0): 1}),
           (("t", 1), ("s", 5), ("t", 0), ("s", 5), {(1, 0): 1}),
           (("t", 0), ("s", 6), ("t", 1), ("s", 6), {(0, 1): 1}),
           (("s", 1), ("s", 1), ("s", 1), ("-", 1), {(1, 0): 1, (1, 1): -1}),
           (("s", 4), ("s", 4), ("s", 4), ("-", 4), {(0, 0): -1, (0, 1): 1})]
_PLAIN = [(("s", j), ("s", j), ("s", j), ("p", j), _CC[j]) for j in _GATHER_ORDER]
_INNER = [_PAIRED if i in _TAIL else _PLAIN for i in range(7)]
_FIRST = [sum(len(x) for x in _INNER[:i]) for i in range(8)]
NZ = _FIRST[7]
MIX = _PLAIN + _PAIRED
MIX_PAIRS = (len(MIX) + 1) // 2
ZH = (NZ + 1) // 2
W3_ROWS = ZH * KS3


def _dft_matrix():
    n = np.arange(LANES)[:, None]
    f = np.arange(LANES)[None, :]
    theta = np.pi * (((4 * f + 1) * n) % (4 * LANES)) / (2 * LANES)
    return np.concatenate([np.cos(theta), -np.sin(theta)], axis=1).astype(jnp.bfloat16)


def _mm(a, b, dims=_NN):
    return lax.dot_general(a, b, dims, preferred_element_type=f32)


def _gelu_scaled(y):
    return y * jnp.tanh(y * (y * y + GELU_C0 / GELU_S)) + y


def _combine(blocks, coef):
    n = len(blocks) // 2
    out = []
    for r in range(n):
        row = []
        for c in range(n):
            acc = None
            for (r0, c0), sign in coef.items():
                v = blocks[r0 * n + r][c0 * n + c]
                acc = v if acc is None else (acc + v if sign > 0 else acc - v)
            row.append(acc)
        out.append(row)
    return out


def _scatter(out, part, coef):
    n = len(part)
    for (r0, c0), sign in coef.items():
        for r in range(n):
            for c in range(n):
                o, v = out[r0 * n + r][c0 * n + c], part[r][c]
                out[r0 * n + r][c0 * n + c] = v if o is None else (o + v if sign > 0 else o - v)


def _gather_steps(get, out, inner=None):
    def one(i):
        part = [[None] * 2 for _ in range(2)]
        for j, spec in enumerate(inner[i] if inner else _PLAIN):
            _scatter(part, [[get(i, j)]], spec[-1])
        _scatter(out, part, _CC[i])
    return [functools.partial(one, i) for i in _GATHER_ORDER]


def _lhs_operands(blocks, tails, specs):
    def operand(kind, j):
        return tails[j] if kind == "t" else _combine(blocks, _AC[j])[0][0]
    out = []
    for low, high, *_ in specs:
        val = operand(*low)
        if high != low:
            val = jnp.concatenate([val[:, :KT], operand(*high)[:, KT:]], axis=1)
        out.append(val.astype(bf16))
    return out


def _rhs_operands(blocks, tails, specs, high):
    def operand(kind, j):
        if kind == "t":
            return tails[j]
        swap = high and kind != "p"
        val = _combine([row[::-1] for row in blocks] if swap else blocks, _BC[j])[0][0]
        return -val if kind == "-" else val
    picks = [spec[3 if high else 2] for spec in specs]
    return [(jnp.zeros_like(tails[0]) if pick is None else operand(*pick)).astype(bf16) for pick in picks]


def _weave(*streams):
    streams = [s for s in streams if s]
    total = [float(sum(w for w, _ in s)) for s in streams]
    pos, done, out = [0] * len(streams), [0.0] * len(streams), []
    while True:
        live = [k for k in range(len(streams)) if pos[k] < len(streams[k])]
        if not live:
            return out
        k = min(live, key=lambda j: (done[j] + 0.5 * streams[j][pos[j]][0]) / total[j])
        out.append(streams[k][pos[k]])
        done[k] += streams[k][pos[k]][0]
        pos[k] += 1


def _weave_groups(*streams):
    woven = _weave(*[[(sum(w for w, _ in grp), grp) for grp in s] for s in streams])
    return [t for _, grp in woven for t in grp]


def _run(tasks):
    for _, fn in tasks:
        fn()


def _kernel(q_hbm, k_hbm, v_hbm, shift_hbm, ssm_hbm, dd_hbm, w1_hbm, w2_hbm, w3_hbm, w4_hbm,
            gw_hbm, dft_hbm, o_hbm,
            q_u, w1_u, w2_u, w3_u, w4_u, shift_v, dd_v, gw_v, o_u,
            k_u, s_u, v_a, v_b, p_a, p_b, sh_a, sh_b,
            w1t_u, w2t_u, dft_u, w1c_u, w2c_u, pcol, gate, x1, xn_u, h1_u, xt_u, xc_u,
            w3c_u, w4c_u,
            acc, z_a, z_b, h_a, h_b, kv_a, kv_b, xf_a, xf_b, kf_a, kf_b, zf_a, zf_b,
            base, sems, idle):
    q_v, w1_v, w2_v, w3_v, w4_v, o_v, w1t, w2t, dft = (
        r.bitcast(bf16) for r in (q_u, w1_u, w2_u, w3_u, w4_u, o_u, w1t_u, w2t_u, dft_u))
    xn, h1, xt = (r.bitcast(bf16) for r in (xn_u, h1_u, xt_u))
    xc = [xc_u.at[pl.ds(t * ZH * TS // 2, ZH * TS // 2), :].bitcast(bf16) for t in range(NT)]
    z = (z_a, z_b)
    h = (h_a.bitcast(bf16), h_b.bitcast(bf16))
    kv = (kv_a.bitcast(bf16), kv_b.bitcast(bf16))
    xf, kf, mb = (xf_a, xf_b), (kf_a, kf_b), (zf_a, zf_b)
    vg = (v_a.bitcast(bf16), v_b.bitcast(bf16))
    pg = (p_a, p_b)
    shifted = (sh_a, sh_b)
    task = functools.partial
    finished = set()

    def need(*tag):
        assert tag in finished, tag

    def rows_at(base, size, align):
        return pl.ds(base if isinstance(base, int) else pl.multiple_of(base, align), size)

    def tile(c):
        return pl.ds(c * LANES, LANES)

    def paired(i, height, offset, size):
        return pl.ds(i // 2 * height + offset, size), tile(i % 2)

    def product(i, offset, size):
        return paired(i, TS, offset, size)

    def chunks(ref_u32, first_row, rows, count):
        window = ref_u32.at[rows_at(first_row, count * (rows // 2), 8), :]
        return [window.at[pl.ds(i * (rows // 2), rows // 2), :].bitcast(bf16) for i in range(count)]

    sem_ids = iter(range(sems.shape[0]))

    def copy(src, dst):
        return pltpu.make_async_copy(src, dst, sems.at[next(sem_ids)])

    cp_q = [copy(q_hbm.at[:, pl.ds(a, b - a)], q_v.at[:, pl.ds(a, b - a)])
            for a, b in ((0, 2 * LANES), (2 * LANES, 4 * LANES), (4 * LANES, 8 * LANES), (8 * LANES, 12 * LANES), (12 * LANES, S))]
    cp_w1 = [copy(w1_hbm.at[:, cols], w1_v.at[:, cols]) for cols in (pl.ds(0, 2 * LANES), pl.ds(2 * LANES, D - 2 * LANES))]
    cp_w2 = copy(w2_hbm, w2_v)
    cp_gate, cp_small = copy(gw_hbm, gw_v), [copy(shift_hbm, shift_v), copy(dd_hbm, dd_v), copy(dft_hbm, dft)]
    sem_w3, sem_w4 = (sems.at[next(sem_ids)] for _ in range(2))
    sem_conv = [[sems.at[next(sem_ids)] for _ in range(2)] for _ in range(2)]
    cp_conv = [copy(k_hbm, k_u.bitcast(bf16)), copy(ssm_hbm, s_u.bitcast(bf16))]
    def put(t, c, r0, r1):
        where = (pl.ds(NB * r0, NB * (r1 - r0)), pl.ds(t * TB + c * NB * LANES, NB * LANES))
        return copy(o_v.at[where], o_hbm.at[where])

    def fetch_w3(f):
        return pltpu.make_async_copy(w3_hbm.at[:, rows_at(f * FC, FC, FC)], w3_v, sem_w3)

    def fetch_w4(f):
        return pltpu.make_async_copy(w4_hbm.at[:, rows_at(f * FC, FC, FC)], w4_v, sem_w4)

    def fetches(s, p):
        g = s + 3
        if isinstance(g, int):
            if not 0 <= g < STEPS:
                return []
            last_v, last_taps = g, g
        else:
            last_v, last_taps = jnp.minimum(g, STEPS - 1), jnp.minimum(g, STEPS)
        return [
            pltpu.make_async_copy(v_hbm.at[rows_at(last_v * CG, CG, CG), :], vg[1 - p], sem_conv[p][0]),
            pltpu.make_async_copy(pcol.at[rows_at(last_taps * CG, CG, CG), pl.ds(0, (KS + 1) * LANES)],
                                  pg[1 - p], sem_conv[p][1])]

    def start(cps):
        for cp in cps:
            cp.start()

    def wait(cps):
        for cp in cps:
            cp.wait()

    def transpose_tasks(src, dst):
        def t(c0, c1):
            dst[c0:c1, :] = jnp.concatenate([src[:, c0:c1], src[KM:D, c0:c1]], axis=0).T
        return [(1, task(t, c0, min(D, c0 + LANES))) for c0 in range(0, D, LANES)]

    def param_tasks():
        def column(j):
            row = (shift_v[j:j + 1, :].astype(f32) if j < KS
                   else (dd_v, gw_v)[j - KS][...].astype(f32).reshape(1, D))
            top = CG if j == KS else 0
            pcol[pl.ds(top, D), tile(j)] = jnp.broadcast_to(row, (LANES, D)).T
            pcol[pl.ds(D - D * (j == KS), CG), tile(j)] = jnp.zeros((CG, LANES), f32)

        def pad():
            zero = jnp.zeros((D // 2, LANES), u32)
            h1_u[:, 0:LANES] = zero
            h1_u[:, LANES + S:] = zero
        return [(1, task(column, KS + 1)), (1, pad)] + [(1, task(column, j)) for j in range(KS + 1)]

    RG = 48
    NG = D // RG

    def fold(x):
        return functools.reduce(lambda u, v: u + v, [x[i:i + 8] for i in range(0, RG, 8)])

    def norm_tasks(c, load, emit):
        st = {"sum": 0.0, "sq": 0.0}

        def sweep1(g):
            st["sum"] = st["sum"] + fold(load(g, True))
            if g == NG - 1:
                st["mean"] = jnp.sum(st["sum"], axis=0, keepdims=True) * (1.0 / D)

        def sweep2(g):
            d = load(g, False) - st["mean"]
            st["sq"] = st["sq"] + fold(d * d)
            if g == NG - 1:
                var = jnp.sum(st["sq"], axis=0, keepdims=True) * (1.0 / D)
                st["rstd"] = lax.rsqrt(var + EPS) * GELU_S

        def sweep3(g):
            emit(g, ((load(g, False) - st["mean"]) * st["rstd"]).astype(bf16))
        return [[(20, task(fn, g)) for g in range(NG)] for fn in (sweep1, sweep2, sweep3)]

    def ln0_tasks(c):
        st = {"logit": 0.0}

        def load(g, first):
            rs = pl.ds(g * RG, RG)
            if not first:
                return x1[rs, tile(c)]
            x = q_v[rs, tile(c)].astype(f32)
            x1[rs, tile(c)] = x
            st["logit"] = st["logit"] + fold(x * pcol[rs, tile(KS + 1)])
            if g == NG - 1:
                logit = jnp.sum(st["logit"], axis=0, keepdims=True)
                gate[:, tile(c)] = jnp.broadcast_to(jax.nn.sigmoid(logit), (8, LANES))
            return x

        def emit(g, val):
            xn[pl.ds(g * RG, RG), tile(c)] = val
            finished.add(("xn", c, g))
        return norm_tasks(c, load, emit)

    def ln1_tasks(c):
        def emit(g, val):
            xn[pl.ds(g * RG, RG), tile(c)] = val
        def load(g, first):
            need("x1", c, g * RG)
            return x1[pl.ds(g * RG, RG), tile(c)]
        return norm_tasks(c, load, emit)

    def to_token_major(c):
        def t():
            tail = xn[KM:D, tile(c)]
            xt[tile(c), :] = jnp.concatenate([xn[:, tile(c)], tail], axis=0).T
        return [(1, t)]

    def mix_tasks(wt, finish, tiles):
        ts, pending = [], []
        for c in tiles:
            for g in range(NB):
                st = {}

                def one(k, c=c, g=g, st=st):
                    k0, k1 = k * LANES, min(D, (k + 1) * LANES)
                    y = _mm(wt[pl.ds(g * DS, DS), k0:k1], xn[k0:k1, tile(c)])
                    st["y"] = y if k == 0 else st["y"] + y
                for k in range(pl.cdiv(D, LANES)):
                    ts.append((DS, task(one, k)))
                    if pending:
                        ts.append((0, pending.pop(0)))
                pending = [task(lambda c, row, st, r: finish(c, row, st["y"][r:r + RG]), c, g * DS + r, st, r)
                           for r in range(0, DS, RG)]
        return ts + [(0, fn) for fn in pending]

    def mix_rhs(pair):
        rows = MIX_PAIRS * LANES
        return (h_a, h_b)[pair % 2].at[pl.ds(pair // 2 * rows // 2, rows // 2), :].bitcast(bf16)

    def mix_lhs_groups(wt, dst):
        dst, half = dst.bitcast(bf16), D // 2

        def t(r, part):
            blk = [[wt[pl.ds(a * half + r, 16), tile(2 * k + part)].astype(f32) for k in range(2)] for a in range(2)]
            tails = [wt[pl.ds(a * half + r, 16), tile(NB)].astype(f32) for a in range(2)]
            for n, val in enumerate(_lhs_operands(blk, tails, (_PLAIN, _PAIRED)[part])):
                dst[paired(part * len(_PLAIN) + n, half, r, 16)] = val
        return [[(40, task(t, r, part))] for r in range(0, half, 16) for part in range(2)]

    def mix_rhs_groups(pair):
        dst = mix_rhs(pair)

        def t(r, part):
            need("xn", 2 * pair + 1, NG - 1)
            blk = [[xn[pl.ds((2 * k + part) * LANES + r, 16), tile(2 * pair + b)].astype(f32)
                    for b in range(2)] for k in range(2)]
            tails = [xn[pl.ds(KM + r % KT, 16), tile(2 * pair + b)].astype(f32) for b in range(2)]
            for n, val in enumerate(_rhs_operands(blk, tails, (_PLAIN, _PAIRED)[part], r >= KT)):
                dst[paired(part * len(_PLAIN) + n, LANES, r, 16)] = val
        return [[(40, task(t, r, part))] for r in range(0, LANES, 16) for part in range(2)]

    def fast_mix_tasks(wc, finish, pairs):
        wc, half = wc.bitcast(bf16), D // 2
        ts, pending = [], []
        for pair in pairs:
            for r in range(0, half, RG):
                out = [[None] * 2 for _ in range(2)]

                def one(n, pair=pair, r=r, out=out):
                    y = _mm(wc[paired(n, half, r, RG)], mix_rhs(pair)[paired(n, LANES, 0, LANES)])
                    _scatter(out, [[y]], MIX[n][-1])
                for n in range(len(MIX)):
                    ts.append((RG, task(one, n)))
                    if pending and n % 2:
                        ts.append((0, pending.pop(0)))
                pending = [task(lambda a, b, r, out, pair: finish(2 * pair + b, a * half + r, out[a][b]), a, b, r, out, pair)
                           for a in range(2) for b in range(2)]
        return ts + [(0, fn) for fn in pending]

    def h1_finish(c, row, y):
        h1[pl.ds(row, RG), tile(c + 1)] = ((0.5 / GELU_S) * _gelu_scaled(y)).astype(bf16)

    def spatial_shift(c):
        rows = D // 8

        def t(g, shift):
            rs = pl.ds(g * rows, rows)
            xn_u[rs, tile(c)] = h1_u[rs, pl.ds((c + 1) * LANES - shift, LANES)]
        return [(1, task(t, g, shift)) for g, shift in enumerate((1, -1, 2, -2))]

    def hs_finish(c, row, y):
        x1[pl.ds(row, RG), tile(c)] += y
        finished.add(("x1", c, row))

    def each(fn, tiles):
        return [t for c in tiles for t in fn(c)]

    def combo_group(load, coef, store):
        blk = [[None] * NB for _ in range(NB)]

        def fetch(a):
            blk[a][:] = [load(a, b) for b in range(NB)]

        def emit(i):
            mid = _combine(blk, coef[i])
            for j in range(7):
                store(7 * i + j, _combine(mid, coef[j])[0][0].astype(bf16))
        return [(20, task(fetch, a)) for a in range(NB)] + [(32, task(emit, i)) for i in range(7)]

    def token(t, b, offset):
        return t * TB + (offset // LANES * NB + b) * LANES + offset % LANES

    def channel(a, offset):
        return (offset // 16 * NB + a) * 16 + offset % 16

    def xc_groups(t):
        out = []
        for r in range(TS // 16):
            blk, tails = [[None] * NB for _ in range(NB)], [None] * NB

            def fetch(b, r=r, blk=blk, tails=tails):
                rs = pl.ds(token(t, b, r * 16), 16)
                blk[b][:] = [xt[rs, tile(k)].astype(f32) for k in range(NB)]
                tails[b] = xt[rs, tile(NB)].astype(f32)

            def emit(i, r=r, blk=blk, tails=tails):
                row = 2 * _TAIL[i][0] if i in _TAIL else 0
                for n, val in enumerate(_lhs_operands(_combine(blk, _AC[i]), tails[row:row + 2], _INNER[i])):
                    xc[t][product(_FIRST[i] + n, r * 16, 16)] = val
            out.append([(22, task(fetch, b)) for b in range(NB)]
                       + [(5 * len(_INNER[i]), task(emit, i)) for i in range(7)])
        return out

    def w3_groups(dst):
        out = []
        for r in range(KS3 // 16):
            high = r >= KT // 16
            blk, tails = [[None] * NB for _ in range(NB)], [None] * NB

            def fetch(k, r=r, blk=blk, tails=tails):
                blk[k][:] = [w3_v[pl.ds(k * KS3 + r * 16, 16), tile(a)].astype(f32) for a in range(NB)]
                tails[k] = w3_v[pl.ds(KM + r * 16 % KT, 16), tile(k)].astype(f32)

            def emit(i, r=r, high=high, blk=blk, tails=tails):
                cols = _TAIL[i][1] if i in _TAIL else (0,)
                sums = [functools.reduce(lambda x, y: x + y, [tails[2 * u + j] for u in cols]) for j in range(2)]
                for n, val in enumerate(_rhs_operands(_combine(blk, _BC[i]), sums, _INNER[i], high)):
                    dst[paired(_FIRST[i] + n, KS3, r * 16, 16)] = val
            out.append([(16, task(fetch, k)) for k in range(NB)]
                       + [(5 * len(_INNER[i]), task(emit, i)) for i in range(7)])
        return out

    def w4_groups(dst):
        out = []
        for r in range(DS // 16):
            def store(i, val, r=r):
                dst[paired(i, DS, r * 16, 16)] = val
            out.append(combo_group(
                lambda a, b, r=r: w4_v[pl.ds(channel(a, r * 16), 16), tile(b)].astype(f32), _AC, store))
        return out

    def clear_tasks(lo, hi):
        def t(n):
            acc[n // NP, n % NP] = jnp.zeros((DS, TS), f32)
        return [(36, task(t, n)) for n in range(lo, hi)]

    def copy_clear_groups(lo, hi):
        def t(n, r):
            acc[n // NP, n % NP, pl.ds(r, RG)] = acc[(n - 1) // NP, (n - 1) % NP, pl.ds(r, RG)]
        return [[(12, task(t, n, r))] for n in range(lo, hi) for r in range(0, DS, RG)]

    def z_tasks(w3c, t):
        m = TS // 4

        def prod(i, r0):
            z[t][product(i, r0, m)] = _mm(xc[t][product(i, r0, m)], w3c[paired(i, KS3, 0, KS3)])
        return [(m, task(prod, i, r0)) for i in range(NZ) for r0 in range(0, TS, m)]

    def act_groups(t):
        out = []
        for r in range(TS // 16):
            grp, halves = [], []
            for r0 in (r * 16, r * 16 + 8):
                pre = [[None] * NB for _ in range(NB)]
                act = [[None] * NB for _ in range(NB)]
                grp += [(24, fn) for fn in _gather_steps(
                    lambda i, j, r0=r0: z[t][product(_FIRST[i] + j, r0, 8)], pre, _INNER)]

                def activate(a, pre=pre, act=act):
                    act[a][:] = [_gelu_scaled(pre[b][a]) for b in range(NB)]
                grp += [(30, task(activate, a)) for a in range(NB)]
                halves.append(act)

            def emit(i, r=r, halves=halves):
                lo, hi = _combine(halves[0], _BC[i]), _combine(halves[1], _BC[i])
                for j in range(7):
                    v = jnp.concatenate([_combine(lo, _BC[j])[0][0], _combine(hi, _BC[j])[0][0]], axis=0)
                    h[t][product(7 * i + j, r * 16, 16)] = v.astype(bf16)
            out.append(grp + [(40, task(emit, i)) for i in range(7)])
        return out

    def w_tasks(w4c, t, by_tile=False):
        def prod(i, c):
            acc[t, i, :, tile(c)] += _mm(w4c[paired(i, DS, 0, DS)], h[t][product(i, c * LANES, LANES)], _NT)
        tiles = range(TS // LANES)
        order = [(i, c) for c in tiles for i in range(NP)] if by_tile else [(i, c) for i in range(NP) for c in tiles]
        return [(DS, task(prod, i, c)) for i, c in order]

    def group_view(ref_u32, row):
        return ref_u32.at[rows_at(row // 2, CG // 2, CG // 2), :]

    def shift_tasks(row, p):
        def t(j):
            words = group_view(k_u, row)[...]
            if j:
                words = pltpu.roll(words, j, axis=1)
                lane = lax.broadcasted_iota(jnp.int32, (CG // 2, LANES), 1)
                shifted[p][pl.ds(j * CG // 2, CG // 2), tile(0)] = jnp.where(lane >= j, words[:, :LANES], 0)
                shifted[p][pl.ds(j * CG // 2, CG // 2), LANES:] = words[:, LANES:]
            else:
                shifted[p][0:CG // 2, :] = words
        return [(1, task(t, j)) for j in range(KS)]

    def kv_groups(p):
        delayed = shifted[p].bitcast(bf16)

        def t(c, r):
            rs = pl.ds(r * 16, 16)
            ksum = None
            for j in range(KS):
                term = delayed[pl.ds(j * CG + r * 16, 16), tile(c)].astype(f32) * pg[p][rs, tile(j)]
                ksum = term if ksum is None else ksum + term
            kv[p][pl.ds(c % (NC // 2) * CG + r * 16, 16), tile(c // (NC // 2))] = (
                ksum * vg[p][rs, tile(c)].astype(f32)).astype(bf16)
        n = 2
        return [[(36, task(t, c, r)) for c in range(c0, c0 + n)] for r in range(CG // 16) for c0 in range(0, NC, n)]

    HALF = NC // 2 * CG

    def data_dft_tasks(p):
        m = HALF // 4

        def t(part, c, r0):
            xf[p][pl.ds(part * HALF + r0, m), tile(c)] = _mm(kv[p][pl.ds(r0, m), tile(part)], dft[:, tile(c)])
        return [(m, task(t, part, c, r0)) for part in range(2) for c in range(2) for r0 in range(0, HALF, m)]

    def filter_dft_tasks(row, p):
        taps = group_view(s_u, row).bitcast(bf16)
        n = NC // 2 // 4

        def t(j0, c):
            lhs = jnp.concatenate([taps[:, tile(j)] for j in range(j0, j0 + n)], axis=0)
            y = _mm(lhs, dft[:, tile(c)])
            if j0 == 0 and c == 0:
                kf[p][0:CG, tile(0)] = y[0:CG] + pg[1 - p][:, tile(KS)]
                kf[p][CG:n * CG, tile(0)] = y[CG:]
            else:
                kf[p][pl.ds(j0 * CG, n * CG), tile(c)] = y
        return [(n * CG, task(t, j0, c)) for j0 in range(0, NC, n) for c in range(2)]

    def mac_groups(p):
        out = []
        block_size = 2
        for u in range(CG // 8):
            full = {}

            def spectrum(ref, j, u=u):
                rs = pl.ds(j * CG + u * 8, 8)
                return ref[rs, tile(0)], ref[rs, tile(1)]

            for i0 in range(0, NC, block_size):
                data = {}

                def add(m, i0=i0, spectrum=spectrum, full=full, data=data):
                    c, d = spectrum(kf[p], m)
                    for i in range(max(i0, m), i0 + block_size):
                        if i - m not in data:
                            data[i - m] = spectrum(xf[p], i - m)
                        a, b = data[i - m]
                        if i in full:
                            full[i] = (full[i][0] + a * c - b * d, full[i][1] + a * d + b * c)
                        else:
                            full[i] = (a * c - b * d, a * d + b * c)

                def finish(i0=i0, u=u, full=full):
                    for i in range(i0, i0 + block_size):
                        re, im = full[i]
                        if i:
                            re, im = re - full[i - 1][1], im + full[i - 1][0]
                        mb[p][pl.ds(i * CG + u * 8, 8), tile(0)] = re
                        mb[p][pl.ds(i * CG + u * 8, 8), tile(1)] = im
                top = i0 + block_size
                out.append([(4 + 8 * (top - max(i0, m)), task(add, m)) for m in range(top)]
                           + [(4 * block_size, finish)])
        return out

    def inverse_dft_tasks(row, p):
        qg, xg, og = (ref.at[rows_at(row, CG, CG), :] for ref in (q_v, x1, base))
        n = 4
        rows = NC * CG // n

        def t(part):
            y = _mm(mb[p][pl.ds(part * rows, rows), :].astype(bf16), dft[...], _NT)
            for j in range(NC // n):
                cs = tile(part * NC // n + j)
                g = jnp.concatenate([gate[:, cs]] * (CG // 8), axis=0)
                conv = y[j * CG:(j + 1) * CG] * qg[:, cs].astype(f32)
                og[:, cs] = (g * (1.0 / LANES)) * conv + (1.0 - g) * xg[:, cs]
        return [(2 * rows, task(t, part)) for part in range(n)]

    def conv_stage(s, p, rows):
        def live(g):
            return not isinstance(g, int) or 0 <= g < STEPS
        mxu, vpu, xlu = [], [], []
        if live(s):
            mxu.append(inverse_dft_tasks(rows[0], p))
        if live(s + 1):
            vpu.append(mac_groups(1 - p))
        if live(s + 2):
            mxu += [filter_dft_tasks(rows[1], p), data_dft_tasks(p)]
        if live(s + 3):
            vpu.append(kv_groups(1 - p))
        if live(s + 4):
            xlu = shift_tasks(rows[2], p)
        return mxu, vpu, xlu

    def out_groups(t, c, r0, r1):
        out = []
        for row in range(r0, r1, 16):
            grp, halves = [], []
            for top in (row, row + 8):
                blk = [[None] * NB for _ in range(NB)]
                grp += [(24, fn) for fn in _gather_steps(
                    lambda i, j, top=top: acc[t, 7 * i + _GATHER_ORDER[j], pl.ds(top, 8), tile(c)], blk)]

                def mix(b, top=top, blk=blk):
                    tok = pl.ds(token(t, b, c * LANES), LANES)
                    scale = (1.0 - gate[:, tok]) * (0.5 / GELU_S)
                    for a in range(NB):
                        blk[a][b] = base[pl.ds(channel(a, top), 8), tok] + scale * blk[a][b]
                grp += [(15, task(mix, b)) for b in range(NB)]
                halves.append(blk)

            def put_rows(b, row=row, halves=halves):
                tok = pl.ds(token(t, b, c * LANES), LANES)
                for a in range(NB):
                    o_v[pl.ds(channel(a, row), 16), tok] = jnp.concatenate(
                        [halves[0][a][b], halves[1][a][b]], axis=0).astype(bf16)
            out.append(grp + [(8, task(put_rows, b)) for b in range(NB)])
        return out

    def block(fn):
        pl.when(pl.semaphore_read(idle) == 0)(fn)

    def compute(mxu=(), vpu=(), xlu=()):
        _run(_weave(_weave(*mxu), _weave_groups(*vpu)) + list(xlu))

    def staggered(fn, tiles):
        sweeps = [fn(c) for c in tiles]
        return [_weave(*[sweeps[i - k][k] for k in range(3) if 0 <= i - k < len(sweeps)])
                for i in range(len(sweeps) + 2)]

    def exchange(done, begin):
        wait(done)
        start(begin)

    def inputs(s, p):
        fetch = (fetch_w3, fetch_w4)[p]
        if isinstance(s, int):
            return fetches(s - 1, 1 - p) + ([fetch(s // NT + 1)] if s > 0 else [])
        return fetches(s - 1, 1 - p) + [fetch(jnp.minimum(s // NT + 1, NF - 1))]

    def group_rows(s):
        clamp = min if isinstance(s, int) else jnp.minimum
        return s * CG, (s + 2) * CG, clamp(s + 4, STEPS - 1) * CG

    def stage(s, p, row, mxu=(), vpu=(), xlu=()):
        m, v, x = conv_stage(s, p, row)
        compute(list(mxu) + m, list(vpu) + v, list(xlu) + x)

    def fixed_stage(s, mxu=(), vpu=(), xlu=(), also=()):
        exchange(inputs(s + 1, 1 - s % 2) + list(also), inputs(s + 2, s % 2))
        block(lambda: stage(s, s % 2, group_rows(s), mxu, vpu, xlu))

    def step(s, p, row3, row4, row_out):
        if p == 0:
            w3c, w3_next = chunks(w3c_u, row3, W3_ROWS, 2)
            w4c, = chunks(w4c_u, row4, W4_ROWS, 1)
            prep = w3_groups(w3_next)
        else:
            w3c, = chunks(w3c_u, row3, W3_ROWS, 1)
            w4c, w4_next = chunks(w4c_u, row4, W4_ROWS, 2)
            prep = w4_groups(w4_next)
        stage(s - 1, 1 - p, row_out, [z_tasks(w3c, 1 - p), w_tasks(w4c, 1 - p)], [act_groups(p), prep])

    def step_rows(s):
        return (s + 1) // NT * (W3_ROWS // 2) + SKEW, (s - 1) // NT * (W4_ROWS // 2) + SKEW, group_rows(s - 1)

    def chunk(ref_u32, f, rows):
        return chunks(ref_u32, f * (rows // 2) + SKEW, rows, 1)[0]

    start([cp_gate, cp_w1[0], cp_q[0], cp_w1[1], cp_q[1]] + cp_small + cp_q[2:]
          + [cp_w2, fetch_w3(0), fetch_w4(0)] + cp_conv)
    c1, c2, c3 = 14, 30, 15
    block(lambda: compute([], [[clear_tasks(0, c1)]]))
    exchange([cp_gate], [])
    block(lambda: compute([], [], param_tasks()[:2]))
    block(lambda: compute([], [[clear_tasks(c1, c1 + 6)]]))
    exchange(cp_w1[:1], [])
    block(lambda: compute([], [], transpose_tasks(w1_v, w1t)[:2]))
    block(lambda: compute([], [[clear_tasks(c1 + 6, c1 + 10)]]))
    exchange([cp_q[0]], [])
    block(lambda: compute([], [staggered(ln0_tasks, range(2))]))
    block(lambda: compute([], [[clear_tasks(c1 + 10, c2)]]))
    exchange(cp_w1[1:], [])
    block(lambda: compute([], [], transpose_tasks(w1_v, w1t)[2:]))

    def first(pairs):
        return fast_mix_tasks(w1c_u, h1_finish, pairs)

    def second(pairs):
        return fast_mix_tasks(w2c_u, hs_finish, pairs)

    def operands(pairs):
        return [grp for pair in pairs for grp in mix_rhs_groups(pair)]

    block(lambda: compute([mix_tasks(w1t, h1_finish, [0])], [mix_lhs_groups(w1t, w1c_u)]))
    exchange([cp_q[1]], [])
    block(lambda: compute([mix_tasks(w1t, h1_finish, [1])], [staggered(ln0_tasks, range(2, 4)) + operands([1])]))
    exchange([cp_q[2]] + cp_small, [])
    block(lambda: compute([first([1])], [staggered(ln0_tasks, range(4, 8)) + operands([2, 3])]))
    exchange([cp_q[3]], [])
    block(lambda: compute([first([2, 3])], [staggered(ln0_tasks, range(8, 12)) + operands([4, 5]),
                                            copy_clear_groups(c2, c2 + c3)]))
    exchange([cp_q[4], cp_w2], [])
    block(lambda: compute([first([4, 5])], [staggered(ln0_tasks, range(12, NC)) + operands([6, 7]),
                                            copy_clear_groups(c2 + c3, c2 + 2 * c3)],
                          transpose_tasks(w2_v, w2t) + each(spatial_shift, range(6))))
    block(lambda: compute([first([6, 7])],
                          [mix_lhs_groups(w2t, w2c_u), operands([0, 1, 2]),
                           copy_clear_groups(c2 + 2 * c3, c2 + 2 * c3 + 8)],
                          each(spatial_shift, range(6, 10))))
    exchange([fetch_w3(0), fetch_w4(0)], [])
    block(lambda: compute([second([0, 1, 2])],
                          [operands([3, 4]), w3_groups(chunk(w3c_u, 0, W3_ROWS)) + w4_groups(chunk(w4c_u, 0, W4_ROWS)),
                           copy_clear_groups(c2 + 2 * c3 + 8, NT * NP)],
                          each(spatial_shift, range(10, NC))))
    exchange([], [fetch_w3(1)])
    block(lambda: compute([second([3, 4])], [operands([5, 6, 7]), staggered(ln1_tasks, range(8))], param_tasks()[2:]))
    block(lambda: compute([second([5])], [staggered(ln1_tasks, range(8, 10))], each(to_token_major, range(8))))
    fixed_stage(-4, [second([6, 7])], [staggered(ln1_tasks, range(10, 12)), xc_groups(0)], also=cp_conv)

    z_first = z_tasks(chunk(w3c_u, 0, W3_ROWS), 0)
    cut, cut1 = len(z_first) * 28 // 100, len(z_first) * 52 // 100
    fixed_stage(-3, [z_first[:cut]], [staggered(ln1_tasks, range(12, NC))], each(to_token_major, range(8, 12)),
                also=[fetch_w3(1)])
    block(lambda: compute([z_first[cut:cut1]], [w3_groups(chunk(w3c_u, 1, W3_ROWS))],
                          each(to_token_major, range(12, NC))))
    fixed_stage(-2, [z_first[cut1:]], [xc_groups(1)])
    fixed_stage(-1, [z_tasks(chunk(w3c_u, 0, W3_ROWS), 1)], [act_groups(0)])

    def body(i, carry):
        for p in (1, 0):
            s = 2 * i + 2 - p
            rows = step_rows(s)
            exchange(inputs(s, p), inputs(s + 1, 1 - p))
            block(task(step, s, p, *rows))
        return carry

    last = STEPS - 2
    lax.fori_loop(0, last // 2, body, 0)

    exchange(inputs(jnp.int32(last + 1), 1), [])
    w4_last = chunk(w4c_u, NF - 1 + pl.semaphore_read(idle), W4_ROWS)
    block(lambda: stage(last, 0, group_rows(last), [w_tasks(w4_last, 0)], [act_groups(1)]))
    w_last = w_tasks(w4_last, 1, by_tile=True)
    pieces = [(0, 0, 0, DS), (0, 1, 0, DS), (1, 0, 0, DS), None, (1, 1, 0, 64), (1, 1, 64, 112), (1, 1, 112, DS)]
    cuts = [0, 26, 52, NP + 30, 2 * NP, 2 * NP, 2 * NP, 2 * NP]
    sent = []
    for n, piece in enumerate(pieces):
        span = w_last[cuts[n]:cuts[n + 1]]
        if n == 0:
            span = inverse_dft_tasks((last + 1) * CG, 1) + span
        block(lambda: compute([span], [out_groups(*piece)] if piece else []))
        if piece:
            sent.append(put(*piece))
            sent[-1].start()
    wait(sent)


@jax.jit
def pallas_gated_mix__ssm_conv_h3__mixer_s_mlp__prompt_kernel(
    A_q: jax.Array,
    A_k: jax.Array,
    A_v: jax.Array,
    A_shift_k: jax.Array,
    A_ssm_k: jax.Array,
    A_ssm_D: jax.Array,
    B_x: jax.Array,
    B_w1: jax.Array,
    B_w2: jax.Array,
    B_w3: jax.Array,
    B_w4: jax.Array,
    gate_w: jax.Array,
):
    del B_x

    def packed(rows, cols, copies=1):
        return [pltpu.VMEM((rows // 2, cols), u32)] * copies

    def wide(*shape, copies=1):
        return [pltpu.VMEM(shape, f32)] * copies

    two = 2 * LANES
    scratch = [
        *packed(D, S), *packed(D, D, 2), *packed(D, FC, 2),
        pltpu.VMEM((KS, D), bf16), pltpu.VMEM((D,), bf16), pltpu.VMEM((D,), bf16),
        *packed(D, S),
        *packed(D, S, 2),
        *packed(CG, S, 2), *wide(CG, (KS + 1) * LANES, copies=2),
        *packed(KS * CG, S, 2),
        *packed(D, KM + LANES, 2), *packed(LANES, two),
        *packed(MIX_PAIRS * D // 2, two, 2),
        *wide(D + CG, (KS + 2) * LANES), *wide(8, S),
        *wide(D, S), *packed(D, S), *packed(D, S + two),
        *packed(S, KM + LANES), *packed(NT * ZH * TS, two),
        *packed((NF + 1) * W3_ROWS + 64, two), *packed(NF * W4_ROWS + 64, two),
        *wide(NT, NP, DS, TS),
        *wide(ZH * TS, two, copies=2), *packed(NH * TS, two, 2),
        *packed(NC * CG // 2, two, 2), *wide(NC * CG, two, copies=6),
        *wide(D, S),
        pltpu.SemaphoreType.DMA((40,)), pltpu.SemaphoreType.REGULAR,
    ]
    hbm = pl.BlockSpec(memory_space=pltpu.HBM)
    out_t = pl.pallas_call(
        _kernel,
        out_shape=jax.ShapeDtypeStruct((D, S), A_q.dtype),
        in_specs=[hbm] * 12,
        out_specs=hbm,
        scratch_shapes=scratch,
        compiler_params=pltpu.CompilerParams(vmem_limit_bytes=124 * 2**20, disable_bounds_checks=True),
        name="gated_mix",
    )(A_q[0].T, A_k[0].T, A_v[0].T, A_shift_k.T, A_ssm_k, A_ssm_D, B_w1, B_w2, B_w3, B_w4.T,
      gate_w, _dft_matrix())
    return out_t.T[None]
```

```python
import functools
import math

import jax
import jax.numpy as jnp
import numpy as np
from jax import lax
from jax.experimental import pallas as pl
from jax.experimental.pallas import tpu as pltpu

S, D, F = 2048, 576, 4608
KS = 4
EPS = 1e-5
LANES = 128

NB, NP = 4, 49
NH = (NP + 1) // 2
FC = 512
NF = F // FC
TB = 1024
NT = S // TB
TS = TB // NB
KM = 512
KT = D - KM
KS3 = KM // NB
DS = D // NB
STEPS = NF * NT
W4_ROWS = -(-NH * DS // 64) * 64
SKEW = 8

NC = S // LANES
CG = D // STEPS

GELU_C0 = math.sqrt(2.0 / math.pi)
GELU_C1 = GELU_C0 * 0.044715
GELU_S = GELU_C1 ** (1.0 / 3.0)

f32, bf16, u32 = jnp.float32, jnp.bfloat16, jnp.uint32
_NN = (((1,), (0,)), ((), ()))
_NT = (((1,), (1,)), ((), ()))

_AC = [{(0, 0): 1, (1, 1): 1}, {(1, 0): 1, (1, 1): 1}, {(0, 0): 1}, {(1, 1): 1},
       {(0, 0): 1, (0, 1): 1}, {(1, 0): 1, (0, 0): -1}, {(0, 1): 1, (1, 1): -1}]
_BC = [{(0, 0): 1, (1, 1): 1}, {(0, 0): 1}, {(0, 1): 1, (1, 1): -1}, {(1, 0): 1, (0, 0): -1},
       {(1, 1): 1}, {(0, 0): 1, (0, 1): 1}, {(1, 0): 1, (1, 1): 1}]
_CC = [{(0, 0): 1, (1, 1): 1}, {(1, 0): 1, (1, 1): -1}, {(0, 1): 1, (1, 1): 1},
       {(0, 0): 1, (1, 0): 1}, {(0, 0): -1, (0, 1): 1}, {(1, 1): 1}, {(0, 0): 1}]
_GATHER_ORDER = (0, 1, 2, 3, 5, 6, 4)
_TAIL = {6: (0, (0, 1)), 5: (1, (0, 1)), 1: (1, (0,)), 4: (0, (1,))}
_PAIRED = [(("s", 0), ("s", 0), ("s", 0), None, {(0, 0): 1, (1, 1): 1}),
           (("s", 0), ("s", 0), None, ("s", 0), {(0, 1): 1, (1, 0): 1}),
           (("s", 2), ("s", 3), ("s", 2), ("s", 3), {(0, 1): 1, (1, 1): 1}),
           (("s", 3), ("s", 2), ("s", 3), ("s", 2), {(0, 0): 1, (1, 0): 1}),
           (("s", 5), ("t", 1), ("s", 5), ("t", 1), {(1, 1): 1}),
           (("s", 6), ("t", 0), ("s", 6), ("t", 0), {(0, 0): 1}),
           (("t", 1), ("s", 5), ("t", 0), ("s", 5), {(1, 0): 1}),
           (("t", 0), ("s", 6), ("t", 1), ("s", 6), {(0, 1): 1}),
           (("s", 1), ("s", 1), ("s", 1), ("-", 1), {(1, 0): 1, (1, 1): -1}),
           (("s", 4), ("s", 4), ("s", 4), ("-", 4), {(0, 0): -1, (0, 1): 1})]
_PLAIN = [(("s", j), ("s", j), ("s", j), ("p", j), _CC[j]) for j in _GATHER_ORDER]
_INNER = [_PAIRED if i in _TAIL else _PLAIN for i in range(7)]
_FIRST = [sum(len(x) for x in _INNER[:i]) for i in range(8)]
NZ = _FIRST[7]
MIX = _PLAIN + _PAIRED
MIX_PAIRS = (len(MIX) + 1) // 2
ZH = (NZ + 1) // 2
W3_ROWS = ZH * KS3


def _dft_matrix():
    n = np.arange(LANES)[:, None]
    f = np.arange(LANES)[None, :]
    theta = np.pi * (((4 * f + 1) * n) % (4 * LANES)) / (2 * LANES)
    return np.concatenate([np.cos(theta), -np.sin(theta)], axis=1).astype(jnp.bfloat16)


def _mm(a, b, dims=_NN):
    return lax.dot_general(a, b, dims, preferred_element_type=f32)


def _gelu_scaled(y):
    return y * jnp.tanh(y * (y * y + GELU_C0 / GELU_S)) + y


def _combine(blocks, coef):
    n = len(blocks) // 2
    out = []
    for r in range(n):
        row = []
        for c in range(n):
            acc = None
            for (r0, c0), sign in coef.items():
                v = blocks[r0 * n + r][c0 * n + c]
                acc = v if acc is None else (acc + v if sign > 0 else acc - v)
            row.append(acc)
        out.append(row)
    return out


def _scatter(out, part, coef):
    n = len(part)
    for (r0, c0), sign in coef.items():
        for r in range(n):
            for c in range(n):
                o, v = out[r0 * n + r][c0 * n + c], part[r][c]
                out[r0 * n + r][c0 * n + c] = v if o is None else (o + v if sign > 0 else o - v)


def _gather_steps(get, out, inner=None):
    def one(i):
        part = [[None] * 2 for _ in range(2)]
        for j, spec in enumerate(inner[i] if inner else _PLAIN):
            _scatter(part, [[get(i, j)]], spec[-1])
        _scatter(out, part, _CC[i])
    return [functools.partial(one, i) for i in _GATHER_ORDER]


def _lhs_operands(blocks, tails, specs):
    def operand(kind, j):
        return tails[j] if kind == "t" else _combine(blocks, _AC[j])[0][0]
    out = []
    for low, high, *_ in specs:
        val = operand(*low)
        if high != low:
            val = jnp.concatenate([val[:, :KT], operand(*high)[:, KT:]], axis=1)
        out.append(val.astype(bf16))
    return out


def _rhs_operands(blocks, tails, specs, high):
    def operand(kind, j):
        if kind == "t":
            return tails[j]
        swap = high and kind != "p"
        val = _combine([row[::-1] for row in blocks] if swap else blocks, _BC[j])[0][0]
        return -val if kind == "-" else val
    picks = [spec[3 if high else 2] for spec in specs]
    return [(jnp.zeros_like(tails[0]) if pick is None else operand(*pick)).astype(bf16) for pick in picks]


def _weave(*streams):
    streams = [s for s in streams if s]
    total = [float(sum(w for w, _ in s)) for s in streams]
    pos, done, out = [0] * len(streams), [0.0] * len(streams), []
    while True:
        live = [k for k in range(len(streams)) if pos[k] < len(streams[k])]
        if not live:
            return out
        k = min(live, key=lambda j: (done[j] + 0.5 * streams[j][pos[j]][0]) / total[j])
        out.append(streams[k][pos[k]])
        done[k] += streams[k][pos[k]][0]
        pos[k] += 1


def _weave_groups(*streams):
    woven = _weave(*[[(sum(w for w, _ in grp), grp) for grp in s] for s in streams])
    return [t for _, grp in woven for t in grp]


def _run(tasks):
    for _, fn in tasks:
        fn()


def _kernel(q_hbm, k_hbm, v_hbm, shift_hbm, ssm_hbm, dd_hbm, w1_hbm, w2_hbm, w3_hbm, w4_hbm,
            gw_hbm, dft_hbm, o_hbm,
            q_u, w1_u, w2_u, w3_u, w4_u, shift_v, dd_v, gw_v, o_u,
            k_u, s_u, v_a, v_b, p_a, p_b, sh_a, sh_b,
            w1t_u, w2t_u, dft_u, w1c_u, w2c_u, pcol, gate, x1, xn_u, h1_u, xt_u, xc_u,
            w3c_u, w4c_u,
            acc, z_a, z_b, h_a, h_b, kv_a, kv_b, xf_a, xf_b, kf_a, kf_b, zf_a, zf_b,
            base, sems, idle):
    q_v, w1_v, w2_v, w3_v, w4_v, o_v, w1t, w2t, dft = (
        r.bitcast(bf16) for r in (q_u, w1_u, w2_u, w3_u, w4_u, o_u, w1t_u, w2t_u, dft_u))
    xn, h1, xt = (r.bitcast(bf16) for r in (xn_u, h1_u, xt_u))
    xc = [xc_u.at[pl.ds(t * ZH * TS // 2, ZH * TS // 2), :].bitcast(bf16) for t in range(NT)]
    z = (z_a, z_b)
    h = (h_a.bitcast(bf16), h_b.bitcast(bf16))
    kv = (kv_a.bitcast(bf16), kv_b.bitcast(bf16))
    xf, kf, mb = (xf_a, xf_b), (kf_a, kf_b), (zf_a, zf_b)
    vg = (v_a.bitcast(bf16), v_b.bitcast(bf16))
    pg = (p_a, p_b)
    shifted = (sh_a, sh_b)
    task = functools.partial
    finished = set()

    def need(*tag):
        assert tag in finished, tag

    def rows_at(base, size, align):
        return pl.ds(base if isinstance(base, int) else pl.multiple_of(base, align), size)

    def tile(c):
        return pl.ds(c * LANES, LANES)

    def paired(i, height, offset, size):
        return pl.ds(i // 2 * height + offset, size), tile(i % 2)

    def product(i, offset, size):
        return paired(i, TS, offset, size)

    def chunks(ref_u32, first_row, rows, count):
        window = ref_u32.at[rows_at(first_row, count * (rows // 2), 8), :]
        return [window.at[pl.ds(i * (rows // 2), rows // 2), :].bitcast(bf16) for i in range(count)]

    sem_ids = iter(range(sems.shape[0]))

    def copy(src, dst):
        return pltpu.make_async_copy(src, dst, sems.at[next(sem_ids)])

    def column_copies(src, dst, edges):
        return [copy(src.at[:, pl.ds(a, b - a)], dst.at[:, pl.ds(a, b - a)]) for a, b in zip(edges, edges[1:])]

    cp_q = column_copies(q_hbm, q_v, [c * LANES for c in (0, 2, 4, 8, 12, NC)])
    cp_w1 = column_copies(w1_hbm, w1_v, [0, 2 * LANES, D])
    cp_w2 = copy(w2_hbm, w2_v)
    cp_gate, cp_small = copy(gw_hbm, gw_v), [copy(shift_hbm, shift_v), copy(dd_hbm, dd_v), copy(dft_hbm, dft)]
    sem_w3, sem_w4 = (sems.at[next(sem_ids)] for _ in range(2))
    sem_conv = [[sems.at[next(sem_ids)] for _ in range(2)] for _ in range(2)]
    cp_conv = [copy(k_hbm, k_u.bitcast(bf16)), copy(ssm_hbm, s_u.bitcast(bf16))]

    def put(t, c, r0, r1):
        where = (pl.ds(NB * r0, NB * (r1 - r0)), pl.ds(t * TB + c * NB * LANES, NB * LANES))
        return copy(o_v.at[where], o_hbm.at[where])

    def fetch_w3(f):
        return pltpu.make_async_copy(w3_hbm.at[:, rows_at(f * FC, FC, FC)], w3_v, sem_w3)

    def fetch_w4(f):
        return pltpu.make_async_copy(w4_hbm.at[:, rows_at(f * FC, FC, FC)], w4_v, sem_w4)

    def fetches(s, p):
        g = s + 3
        if isinstance(g, int):
            if not 0 <= g < STEPS:
                return []
            last_v, last_taps = g, g
        else:
            last_v, last_taps = jnp.minimum(g, STEPS - 1), jnp.minimum(g, STEPS)
        return [
            pltpu.make_async_copy(v_hbm.at[rows_at(last_v * CG, CG, CG), :], vg[1 - p], sem_conv[p][0]),
            pltpu.make_async_copy(pcol.at[rows_at(last_taps * CG, CG, CG), pl.ds(0, (KS + 1) * LANES)],
                                  pg[1 - p], sem_conv[p][1])]

    def start(cps):
        for cp in cps:
            cp.start()

    def wait(cps):
        for cp in cps:
            cp.wait()

    def transpose_tasks(src, dst):
        def t(c0, c1):
            dst[c0:c1, :] = jnp.concatenate([src[:, c0:c1], src[KM:D, c0:c1]], axis=0).T
        return [(1, task(t, c0, min(D, c0 + LANES))) for c0 in range(0, D, LANES)]

    def param_tasks():
        def column(j):
            row = (shift_v[j:j + 1, :].astype(f32) if j < KS
                   else (dd_v, gw_v)[j - KS][...].astype(f32).reshape(1, D))
            top = CG if j == KS else 0
            pcol[pl.ds(top, D), tile(j)] = jnp.broadcast_to(row, (LANES, D)).T
            pcol[pl.ds(D - D * (j == KS), CG), tile(j)] = jnp.zeros((CG, LANES), f32)

        def pad():
            zero = jnp.zeros((D // 2, LANES), u32)
            h1_u[:, 0:LANES] = zero
            h1_u[:, LANES + S:] = zero
        return [(1, task(column, KS + 1)), (1, pad)] + [(1, task(column, j)) for j in range(KS + 1)]

    RG = 48
    NG = D // RG

    def fold(x):
        return functools.reduce(lambda u, v: u + v, [x[i:i + 8] for i in range(0, RG, 8)])

    def norm_tasks(c, load, emit):
        st = {"sum": 0.0, "sq": 0.0}

        def sweep1(g):
            st["sum"] = st["sum"] + fold(load(g, True))
            if g == NG - 1:
                st["mean"] = jnp.sum(st["sum"], axis=0, keepdims=True) * (1.0 / D)

        def sweep2(g):
            d = load(g, False) - st["mean"]
            st["sq"] = st["sq"] + fold(d * d)
            if g == NG - 1:
                var = jnp.sum(st["sq"], axis=0, keepdims=True) * (1.0 / D)
                st["rstd"] = lax.rsqrt(var + EPS) * GELU_S

        def sweep3(g):
            emit(g, ((load(g, False) - st["mean"]) * st["rstd"]).astype(bf16))
        return [[(20, task(fn, g)) for g in range(NG)] for fn in (sweep1, sweep2, sweep3)]

    def ln0_tasks(c):
        st = {"logit": 0.0}

        def load(g, first):
            rs = pl.ds(g * RG, RG)
            if not first:
                return x1[rs, tile(c)]
            x = q_v[rs, tile(c)].astype(f32)
            x1[rs, tile(c)] = x
            st["logit"] = st["logit"] + fold(x * pcol[rs, tile(KS + 1)])
            if g == NG - 1:
                logit = jnp.sum(st["logit"], axis=0, keepdims=True)
                gate[:, tile(c)] = jnp.broadcast_to(jax.nn.sigmoid(logit), (8, LANES))
            return x

        def emit(g, val):
            xn[pl.ds(g * RG, RG), tile(c)] = val
            finished.add(("xn", c, g))
        return norm_tasks(c, load, emit)

    def ln1_tasks(c):
        def emit(g, val):
            xn[pl.ds(g * RG, RG), tile(c)] = val
        def load(g, first):
            need("x1", c, g * RG)
            return x1[pl.ds(g * RG, RG), tile(c)]
        return norm_tasks(c, load, emit)

    def to_token_major(c):
        def t():
            tail = xn[KM:D, tile(c)]
            xt[tile(c), :] = jnp.concatenate([xn[:, tile(c)], tail], axis=0).T
        return [(1, t)]

    def mix_tasks(wt, finish, tiles):
        ts, pending = [], []
        for c in tiles:
            for g in range(NB):
                st = {}

                def one(k, c=c, g=g, st=st):
                    k0, k1 = k * LANES, min(D, (k + 1) * LANES)
                    y = _mm(wt[pl.ds(g * DS, DS), k0:k1], xn[k0:k1, tile(c)])
                    st["y"] = y if k == 0 else st["y"] + y
                for k in range(pl.cdiv(D, LANES)):
                    ts.append((DS, task(one, k)))
                    if pending:
                        ts.append((0, pending.pop(0)))
                pending = [task(lambda c, row, st, r: finish(c, row, st["y"][r:r + RG]), c, g * DS + r, st, r)
                           for r in range(0, DS, RG)]
        return ts + [(0, fn) for fn in pending]

    def mix_rhs(pair):
        rows = MIX_PAIRS * LANES
        return (h_a, h_b)[pair % 2].at[pl.ds(pair // 2 * rows // 2, rows // 2), :].bitcast(bf16)

    def mix_lhs_groups(wt, dst):
        dst, half = dst.bitcast(bf16), D // 2

        def t(r, part):
            blk = [[wt[pl.ds(a * half + r, 16), tile(2 * k + part)].astype(f32) for k in range(2)] for a in range(2)]
            tails = [wt[pl.ds(a * half + r, 16), tile(NB)].astype(f32) for a in range(2)]
            for n, val in enumerate(_lhs_operands(blk, tails, (_PLAIN, _PAIRED)[part])):
                dst[paired(part * len(_PLAIN) + n, half, r, 16)] = val
        return [[(40, task(t, r, part))] for r in range(0, half, 16) for part in range(2)]

    def mix_rhs_groups(pair):
        dst = mix_rhs(pair)

        def t(r, part):
            need("xn", 2 * pair + 1, NG - 1)
            blk = [[xn[pl.ds((2 * k + part) * LANES + r, 16), tile(2 * pair + b)].astype(f32)
                    for b in range(2)] for k in range(2)]
            tails = [xn[pl.ds(KM + r % KT, 16), tile(2 * pair + b)].astype(f32) for b in range(2)]
            for n, val in enumerate(_rhs_operands(blk, tails, (_PLAIN, _PAIRED)[part], r >= KT)):
                dst[paired(part * len(_PLAIN) + n, LANES, r, 16)] = val
        return [[(40, task(t, r, part))] for r in range(0, LANES, 16) for part in range(2)]

    def fast_mix_tasks(wc, finish, pairs):
        wc, half = wc.bitcast(bf16), D // 2
        ts, pending = [], []
        for pair in pairs:
            for r in range(0, half, RG):
                out = [[None] * 2 for _ in range(2)]

                def one(n, pair=pair, r=r, out=out):
                    y = _mm(wc[paired(n, half, r, RG)], mix_rhs(pair)[paired(n, LANES, 0, LANES)])
                    _scatter(out, [[y]], MIX[n][-1])
                for n in range(len(MIX)):
                    ts.append((RG, task(one, n)))
                    if pending and n % 2:
                        ts.append((0, pending.pop(0)))
                pending = [task(lambda a, b, r, out, pair: finish(2 * pair + b, a * half + r, out[a][b]), a, b, r, out, pair)
                           for a in range(2) for b in range(2)]
        return ts + [(0, fn) for fn in pending]

    def h1_finish(c, row, y):
        h1[pl.ds(row, RG), tile(c + 1)] = ((0.5 / GELU_S) * _gelu_scaled(y)).astype(bf16)

    def spatial_shift(c):
        rows = D // 8

        def t(g, shift):
            rs = pl.ds(g * rows, rows)
            xn_u[rs, tile(c)] = h1_u[rs, pl.ds((c + 1) * LANES - shift, LANES)]
        return [(1, task(t, g, shift)) for g, shift in enumerate((1, -1, 2, -2))]

    def hs_finish(c, row, y):
        x1[pl.ds(row, RG), tile(c)] += y
        finished.add(("x1", c, row))

    def each(fn, tiles):
        return [t for c in tiles for t in fn(c)]

    def combo_group(load, coef, store):
        blk = [[None] * NB for _ in range(NB)]

        def fetch(a):
            blk[a][:] = [load(a, b) for b in range(NB)]

        def emit(i):
            mid = _combine(blk, coef[i])
            for j in range(7):
                store(7 * i + j, _combine(mid, coef[j])[0][0].astype(bf16))
        return [(20, task(fetch, a)) for a in range(NB)] + [(32, task(emit, i)) for i in range(7)]

    def token(t, b, offset):
        return t * TB + (offset // LANES * NB + b) * LANES + offset % LANES

    def channel(a, offset):
        return (offset // 16 * NB + a) * 16 + offset % 16

    def xc_groups(t):
        out = []
        for r in range(TS // 16):
            blk, tails = [[None] * NB for _ in range(NB)], [None] * NB

            def fetch(b, r=r, blk=blk, tails=tails):
                rs = pl.ds(token(t, b, r * 16), 16)
                blk[b][:] = [xt[rs, tile(k)].astype(f32) for k in range(NB)]
                tails[b] = xt[rs, tile(NB)].astype(f32)

            def emit(i, r=r, blk=blk, tails=tails):
                row = 2 * _TAIL[i][0] if i in _TAIL else 0
                for n, val in enumerate(_lhs_operands(_combine(blk, _AC[i]), tails[row:row + 2], _INNER[i])):
                    xc[t][product(_FIRST[i] + n, r * 16, 16)] = val
            out.append([(22, task(fetch, b)) for b in range(NB)]
                       + [(5 * len(_INNER[i]), task(emit, i)) for i in range(7)])
        return out

    def w3_groups(dst):
        out = []
        for r in range(KS3 // 16):
            high = r >= KT // 16
            blk, tails = [[None] * NB for _ in range(NB)], [None] * NB

            def fetch(k, r=r, blk=blk, tails=tails):
                blk[k][:] = [w3_v[pl.ds(k * KS3 + r * 16, 16), tile(a)].astype(f32) for a in range(NB)]
                tails[k] = w3_v[pl.ds(KM + r * 16 % KT, 16), tile(k)].astype(f32)

            def emit(i, r=r, high=high, blk=blk, tails=tails):
                cols = _TAIL[i][1] if i in _TAIL else (0,)
                sums = [functools.reduce(lambda x, y: x + y, [tails[2 * u + j] for u in cols]) for j in range(2)]
                for n, val in enumerate(_rhs_operands(_combine(blk, _BC[i]), sums, _INNER[i], high)):
                    dst[paired(_FIRST[i] + n, KS3, r * 16, 16)] = val
            out.append([(16, task(fetch, k)) for k in range(NB)]
                       + [(5 * len(_INNER[i]), task(emit, i)) for i in range(7)])
        return out

    def w4_groups(dst):
        out = []
        for r in range(DS // 16):
            def store(i, val, r=r):
                dst[paired(i, DS, r * 16, 16)] = val
            out.append(combo_group(
                lambda a, b, r=r: w4_v[pl.ds(channel(a, r * 16), 16), tile(b)].astype(f32), _AC, store))
        return out

    def clear_tasks(lo, hi):
        def t(n):
            acc[n // NP, n % NP] = jnp.zeros((DS, TS), f32)
        return [(36, task(t, n)) for n in range(lo, hi)]

    def copy_clear_groups(lo, hi):
        def t(n, r):
            acc[n // NP, n % NP, pl.ds(r, RG)] = acc[(n - 1) // NP, (n - 1) % NP, pl.ds(r, RG)]
        return [[(12, task(t, n, r))] for n in range(lo, hi) for r in range(0, DS, RG)]

    def z_tasks(w3c, t):
        m = TS // 4

        def prod(i, r0):
            z[t][product(i, r0, m)] = _mm(xc[t][product(i, r0, m)], w3c[paired(i, KS3, 0, KS3)])
        return [(m, task(prod, i, r0)) for i in range(NZ) for r0 in range(0, TS, m)]

    def act_groups(t):
        out = []
        for r in range(TS // 16):
            grp, halves = [], []
            for r0 in (r * 16, r * 16 + 8):
                pre = [[None] * NB for _ in range(NB)]
                act = [[None] * NB for _ in range(NB)]
                grp += [(24, fn) for fn in _gather_steps(
                    lambda i, j, r0=r0: z[t][product(_FIRST[i] + j, r0, 8)], pre, _INNER)]

                def activate(a, pre=pre, act=act):
                    act[a][:] = [_gelu_scaled(pre[b][a]) for b in range(NB)]
                grp += [(30, task(activate, a)) for a in range(NB)]
                halves.append(act)

            def emit(i, r=r, halves=halves):
                lo, hi = _combine(halves[0], _BC[i]), _combine(halves[1], _BC[i])
                for j in range(7):
                    v = jnp.concatenate([_combine(lo, _BC[j])[0][0], _combine(hi, _BC[j])[0][0]], axis=0)
                    h[t][product(7 * i + j, r * 16, 16)] = v.astype(bf16)
            out.append(grp + [(40, task(emit, i)) for i in range(7)])
        return out

    def w_tasks(w4c, t, by_tile=False):
        def prod(i, c):
            acc[t, i, :, tile(c)] += _mm(w4c[paired(i, DS, 0, DS)], h[t][product(i, c * LANES, LANES)], _NT)
        tiles = range(TS // LANES)
        order = [(i, c) for c in tiles for i in range(NP)] if by_tile else [(i, c) for i in range(NP) for c in tiles]
        return [(DS, task(prod, i, c)) for i, c in order]

    def group_view(ref_u32, row):
        return ref_u32.at[rows_at(row // 2, CG // 2, CG // 2), :]

    def shift_tasks(row, p):
        def t(j):
            words = group_view(k_u, row)[...]
            if j:
                words = pltpu.roll(words, j, axis=1)
                lane = lax.broadcasted_iota(jnp.int32, (CG // 2, LANES), 1)
                shifted[p][pl.ds(j * CG // 2, CG // 2), tile(0)] = jnp.where(lane >= j, words[:, :LANES], 0)
                shifted[p][pl.ds(j * CG // 2, CG // 2), LANES:] = words[:, LANES:]
            else:
                shifted[p][0:CG // 2, :] = words
        return [(1, task(t, j)) for j in range(KS)]

    def kv_groups(p):
        delayed = shifted[p].bitcast(bf16)

        def t(c, r):
            rs = pl.ds(r * 16, 16)
            ksum = None
            for j in range(KS):
                term = delayed[pl.ds(j * CG + r * 16, 16), tile(c)].astype(f32) * pg[p][rs, tile(j)]
                ksum = term if ksum is None else ksum + term
            kv[p][pl.ds(c % (NC // 2) * CG + r * 16, 16), tile(c // (NC // 2))] = (
                ksum * vg[p][rs, tile(c)].astype(f32)).astype(bf16)
        n = 2
        return [[(36, task(t, c, r)) for c in range(c0, c0 + n)] for r in range(CG // 16) for c0 in range(0, NC, n)]

    HALF = NC // 2 * CG

    def data_dft_tasks(p):
        m = HALF // 4

        def t(part, c, r0):
            xf[p][pl.ds(part * HALF + r0, m), tile(c)] = _mm(kv[p][pl.ds(r0, m), tile(part)], dft[:, tile(c)])
        return [(m, task(t, part, c, r0)) for part in range(2) for c in range(2) for r0 in range(0, HALF, m)]

    def filter_dft_tasks(row, p):
        taps = group_view(s_u, row).bitcast(bf16)
        n = NC // 2 // 4

        def t(j0, c):
            lhs = jnp.concatenate([taps[:, tile(j)] for j in range(j0, j0 + n)], axis=0)
            y = _mm(lhs, dft[:, tile(c)])
            if j0 == 0 and c == 0:
                kf[p][0:CG, tile(0)] = y[0:CG] + pg[1 - p][:, tile(KS)]
                kf[p][CG:n * CG, tile(0)] = y[CG:]
            else:
                kf[p][pl.ds(j0 * CG, n * CG), tile(c)] = y
        return [(n * CG, task(t, j0, c)) for j0 in range(0, NC, n) for c in range(2)]

    def mac_groups(p):
        out = []
        block_size = 2
        for u in range(CG // 8):
            full = {}

            def spectrum(ref, j, u=u):
                rs = pl.ds(j * CG + u * 8, 8)
                return ref[rs, tile(0)], ref[rs, tile(1)]

            for i0 in range(0, NC, block_size):
                data = {}

                def add(m, i0=i0, spectrum=spectrum, full=full, data=data):
                    c, d = spectrum(kf[p], m)
                    for i in range(max(i0, m), i0 + block_size):
                        if i - m not in data:
                            data[i - m] = spectrum(xf[p], i - m)
                        a, b = data[i - m]
                        if i in full:
                            full[i] = (full[i][0] + a * c - b * d, full[i][1] + a * d + b * c)
                        else:
                            full[i] = (a * c - b * d, a * d + b * c)

                def finish(i0=i0, u=u, full=full):
                    for i in range(i0, i0 + block_size):
                        re, im = full[i]
                        if i:
                            re, im = re - full[i - 1][1], im + full[i - 1][0]
                        mb[p][pl.ds(i * CG + u * 8, 8), tile(0)] = re
                        mb[p][pl.ds(i * CG + u * 8, 8), tile(1)] = im
                top = i0 + block_size
                out.append([(4 + 8 * (top - max(i0, m)), task(add, m)) for m in range(top)]
                           + [(4 * block_size, finish)])
        return out

    def inverse_dft_tasks(row, p):
        qg, xg, og = (ref.at[rows_at(row, CG, CG), :] for ref in (q_v, x1, base))
        n = 4
        rows = NC * CG // n

        def t(part):
            y = _mm(mb[p][pl.ds(part * rows, rows), :].astype(bf16), dft[...], _NT)
            for j in range(NC // n):
                cs = tile(part * NC // n + j)
                g = jnp.concatenate([gate[:, cs]] * (CG // 8), axis=0)
                conv = y[j * CG:(j + 1) * CG] * qg[:, cs].astype(f32)
                og[:, cs] = (g * (1.0 / LANES)) * conv + (1.0 - g) * xg[:, cs]
        return [(2 * rows, task(t, part)) for part in range(n)]

    def conv_stage(s, p, rows):
        def live(g):
            return not isinstance(g, int) or 0 <= g < STEPS
        mxu, vpu, xlu = [], [], []
        if live(s):
            mxu.append(inverse_dft_tasks(rows[0], p))
        if live(s + 1):
            vpu.append(mac_groups(1 - p))
        if live(s + 2):
            mxu += [filter_dft_tasks(rows[1], p), data_dft_tasks(p)]
        if live(s + 3):
            vpu.append(kv_groups(1 - p))
        if live(s + 4):
            xlu = shift_tasks(rows[2], p)
        return mxu, vpu, xlu

    def out_groups(t, c, r0, r1):
        out = []
        for row in range(r0, r1, 16):
            grp, halves = [], []
            for top in (row, row + 8):
                blk = [[None] * NB for _ in range(NB)]
                grp += [(24, fn) for fn in _gather_steps(
                    lambda i, j, top=top: acc[t, 7 * i + _GATHER_ORDER[j], pl.ds(top, 8), tile(c)], blk)]

                def mix(b, top=top, blk=blk):
                    tok = pl.ds(token(t, b, c * LANES), LANES)
                    scale = (1.0 - gate[:, tok]) * (0.5 / GELU_S)
                    for a in range(NB):
                        blk[a][b] = base[pl.ds(channel(a, top), 8), tok] + scale * blk[a][b]
                grp += [(15, task(mix, b)) for b in range(NB)]
                halves.append(blk)

            def put_rows(b, row=row, halves=halves):
                tok = pl.ds(token(t, b, c * LANES), LANES)
                for a in range(NB):
                    o_v[pl.ds(channel(a, row), 16), tok] = jnp.concatenate(
                        [halves[0][a][b], halves[1][a][b]], axis=0).astype(bf16)
            out.append(grp + [(8, task(put_rows, b)) for b in range(NB)])
        return out

    def block(fn):
        pl.when(pl.semaphore_read(idle) == 0)(fn)

    def compute(mxu=(), vpu=(), xlu=()):
        _run(_weave(_weave(*mxu), _weave_groups(*vpu)) + list(xlu))

    def staggered(fn, tiles):
        sweeps = [fn(c) for c in tiles]
        return [_weave(*[sweeps[i - k][k] for k in range(3) if 0 <= i - k < len(sweeps)])
                for i in range(len(sweeps) + 2)]

    def exchange(done, begin):
        wait(done)
        start(begin)

    def inputs(s, p):
        fetch = (fetch_w3, fetch_w4)[p]
        if isinstance(s, int):
            return fetches(s - 1, 1 - p) + ([fetch(s // NT + 1)] if s > 0 else [])
        return fetches(s - 1, 1 - p) + [fetch(jnp.minimum(s // NT + 1, NF - 1))]

    def group_rows(s):
        clamp = min if isinstance(s, int) else jnp.minimum
        return s * CG, (s + 2) * CG, clamp(s + 4, STEPS - 1) * CG

    def stage(s, p, rows, mxu=(), vpu=(), xlu=()):
        m, v, x = conv_stage(s, p, rows)
        compute(list(mxu) + m, list(vpu) + v, list(xlu) + x)

    def fixed_stage(s, mxu=(), vpu=(), xlu=(), also=()):
        exchange(inputs(s + 1, 1 - s % 2) + list(also), inputs(s + 2, s % 2))
        block(lambda: stage(s, s % 2, group_rows(s), mxu, vpu, xlu))

    def step(s, p, row3, row4, rows):
        if p == 0:
            w3c, w3_next = chunks(w3c_u, row3, W3_ROWS, 2)
            w4c, = chunks(w4c_u, row4, W4_ROWS, 1)
            prep = w3_groups(w3_next)
        else:
            w3c, = chunks(w3c_u, row3, W3_ROWS, 1)
            w4c, w4_next = chunks(w4c_u, row4, W4_ROWS, 2)
            prep = w4_groups(w4_next)
        stage(s - 1, 1 - p, rows, [z_tasks(w3c, 1 - p), w_tasks(w4c, 1 - p)], [act_groups(p), prep])

    def step_rows(s):
        return (s + 1) // NT * (W3_ROWS // 2) + SKEW, (s - 1) // NT * (W4_ROWS // 2) + SKEW, group_rows(s - 1)

    def chunk(ref_u32, f, rows):
        return chunks(ref_u32, f * (rows // 2) + SKEW, rows, 1)[0]

    start([cp_gate, cp_w1[0], cp_q[0], cp_w1[1], cp_q[1]] + cp_small + cp_q[2:]
          + [cp_w2, fetch_w3(0), fetch_w4(0)] + cp_conv)
    c1, c2, c3 = 14, 30, 15
    block(lambda: compute([], [[clear_tasks(0, c1)]]))
    exchange([cp_gate], [])
    block(lambda: compute([], [], param_tasks()[:2]))
    block(lambda: compute([], [[clear_tasks(c1, c1 + 6)]]))
    exchange(cp_w1[:1], [])
    block(lambda: compute([], [], transpose_tasks(w1_v, w1t)[:2]))
    block(lambda: compute([], [[clear_tasks(c1 + 6, c1 + 10)]]))
    exchange([cp_q[0]], [])
    block(lambda: compute([], [staggered(ln0_tasks, range(2))]))
    block(lambda: compute([], [[clear_tasks(c1 + 10, c2)]]))
    exchange(cp_w1[1:], [])
    block(lambda: compute([], [], transpose_tasks(w1_v, w1t)[2:]))

    def first(pairs):
        return fast_mix_tasks(w1c_u, h1_finish, pairs)

    def second(pairs):
        return fast_mix_tasks(w2c_u, hs_finish, pairs)

    def operands(pairs):
        return [grp for pair in pairs for grp in mix_rhs_groups(pair)]

    block(lambda: compute([mix_tasks(w1t, h1_finish, [0])], [mix_lhs_groups(w1t, w1c_u)]))
    exchange([cp_q[1]], [])
    block(lambda: compute([mix_tasks(w1t, h1_finish, [1])], [staggered(ln0_tasks, range(2, 4)) + operands([1])]))
    exchange([cp_q[2]] + cp_small, [])
    block(lambda: compute([first([1])], [staggered(ln0_tasks, range(4, 8)) + operands([2, 3])]))
    exchange([cp_q[3]], [])
    block(lambda: compute([first([2, 3])], [staggered(ln0_tasks, range(8, 12)) + operands([4, 5]),
                                            copy_clear_groups(c2, c2 + c3)]))
    exchange([cp_q[4], cp_w2], [])
    block(lambda: compute([first([4, 5])], [staggered(ln0_tasks, range(12, NC)) + operands([6, 7]),
                                            copy_clear_groups(c2 + c3, c2 + 2 * c3)],
                          transpose_tasks(w2_v, w2t) + each(spatial_shift, range(6))))
    block(lambda: compute([first([6, 7])],
                          [mix_lhs_groups(w2t, w2c_u), operands([0, 1, 2]),
                           copy_clear_groups(c2 + 2 * c3, c2 + 2 * c3 + 8)],
                          each(spatial_shift, range(6, 10))))
    exchange([fetch_w3(0), fetch_w4(0)], [])
    block(lambda: compute([second([0, 1, 2])],
                          [operands([3, 4]), w3_groups(chunk(w3c_u, 0, W3_ROWS)) + w4_groups(chunk(w4c_u, 0, W4_ROWS)),
                           copy_clear_groups(c2 + 2 * c3 + 8, NT * NP)],
                          each(spatial_shift, range(10, NC))))
    exchange([], [fetch_w3(1)])
    block(lambda: compute([second([3, 4])], [operands([5, 6, 7]), staggered(ln1_tasks, range(8))], param_tasks()[2:]))
    block(lambda: compute([second([5])], [staggered(ln1_tasks, range(8, 10))], each(to_token_major, range(8))))
    fixed_stage(-4, [second([6, 7])], [staggered(ln1_tasks, range(10, 12)), xc_groups(0)], also=cp_conv)

    z_first = z_tasks(chunk(w3c_u, 0, W3_ROWS), 0)
    cut, cut1 = len(z_first) * 28 // 100, len(z_first) * 52 // 100
    fixed_stage(-3, [z_first[:cut]], [staggered(ln1_tasks, range(12, NC))], each(to_token_major, range(8, 12)),
                also=[fetch_w3(1)])
    block(lambda: compute([z_first[cut:cut1]], [w3_groups(chunk(w3c_u, 1, W3_ROWS))],
                          each(to_token_major, range(12, NC))))
    fixed_stage(-2, [z_first[cut1:]], [xc_groups(1)])
    fixed_stage(-1, [z_tasks(chunk(w3c_u, 0, W3_ROWS), 1)], [act_groups(0)])

    def body(i, carry):
        for p in (1, 0):
            s = 2 * i + 2 - p
            rows = step_rows(s)
            exchange(inputs(s, p), inputs(s + 1, 1 - p))
            block(task(step, s, p, *rows))
        return carry

    last = STEPS - 2
    lax.fori_loop(0, last // 2, body, 0)

    exchange(inputs(jnp.int32(last + 1), 1), [])
    w4_last = chunk(w4c_u, NF - 1, W4_ROWS)
    block(lambda: stage(last, 0, group_rows(last), [w_tasks(w4_last, 0)], [act_groups(1)]))
    w_last = w_tasks(w4_last, 1, by_tile=True)
    pieces = [(0, 0, 0, DS), (0, 1, 0, DS), (1, 0, 0, DS), None, (1, 1, 0, 64), (1, 1, 64, 112), (1, 1, 112, DS)]
    cuts = [0, 26, 52, NP + 30, 2 * NP, 2 * NP, 2 * NP, 2 * NP]
    sent = []
    for n, piece in enumerate(pieces):
        span = w_last[cuts[n]:cuts[n + 1]]
        if n == 0:
            span = inverse_dft_tasks((last + 1) * CG, 1) + span
        block(lambda: compute([span], [out_groups(*piece)] if piece else []))
        if piece:
            sent.append(put(*piece))
            sent[-1].start()
    wait(sent)


@jax.jit
def pallas_gated_mix__ssm_conv_h3__mixer_s_mlp__prompt_kernel(
    A_q: jax.Array,
    A_k: jax.Array,
    A_v: jax.Array,
    A_shift_k: jax.Array,
    A_ssm_k: jax.Array,
    A_ssm_D: jax.Array,
    B_x: jax.Array,
    B_w1: jax.Array,
    B_w2: jax.Array,
    B_w3: jax.Array,
    B_w4: jax.Array,
    gate_w: jax.Array,
):
    del B_x

    def packed(rows, cols, copies=1):
        return [pltpu.VMEM((rows // 2, cols), u32)] * copies

    def wide(*shape, copies=1):
        return [pltpu.VMEM(shape, f32)] * copies

    two = 2 * LANES
    scratch = [
        *packed(D, S), *packed(D, D, 2), *packed(D, FC, 2),
        pltpu.VMEM((KS, D), bf16), pltpu.VMEM((D,), bf16), pltpu.VMEM((D,), bf16),
        *packed(D, S),
        *packed(D, S, 2),
        *packed(CG, S, 2), *wide(CG, (KS + 1) * LANES, copies=2),
        *packed(KS * CG, S, 2),
        *packed(D, KM + LANES, 2), *packed(LANES, two),
        *packed(MIX_PAIRS * D // 2, two, 2),
        *wide(D + CG, (KS + 2) * LANES), *wide(8, S),
        *wide(D, S), *packed(D, S), *packed(D, S + two),
        *packed(S, KM + LANES), *packed(NT * ZH * TS, two),
        *packed((NF + 1) * W3_ROWS + 64, two), *packed(NF * W4_ROWS + 64, two),
        *wide(NT, NP, DS, TS),
        *wide(ZH * TS, two, copies=2), *packed(NH * TS, two, 2),
        *packed(NC * CG // 2, two, 2), *wide(NC * CG, two, copies=6),
        *wide(D, S),
        pltpu.SemaphoreType.DMA((40,)), pltpu.SemaphoreType.REGULAR,
    ]
    hbm = pl.BlockSpec(memory_space=pltpu.HBM)
    out_t = pl.pallas_call(
        _kernel,
        out_shape=jax.ShapeDtypeStruct((D, S), A_q.dtype),
        in_specs=[hbm] * 12,
        out_specs=hbm,
        scratch_shapes=scratch,
        compiler_params=pltpu.CompilerParams(vmem_limit_bytes=124 * 2**20, disable_bounds_checks=True),
        name="gated_mix",
    )(A_q[0].T, A_k[0].T, A_v[0].T, A_shift_k.T, A_ssm_k, A_ssm_D, B_w1, B_w2, B_w3, B_w4.T,
      gate_w, _dft_matrix())
    return out_t.T[None]
```
